```python
import os as _os
_os.environ.setdefault("JAX_PLATFORMS", "cpu")
import jax
import jax.numpy as jnp

def _softmax(x, axis=-1):
    return jax.nn.softmax(x, axis=axis)
def _gelu(x):
    return jax.nn.gelu(x, approximate=True)
def _silu(x):
    return jax.nn.silu(x)
def _sigmoid(x):
    return jax.nn.sigmoid(x)
def _layernorm(x, axis=-1, eps=1e-5):
    m = jnp.mean(x, axis=axis, keepdims=True)
    v = jnp.var(x, axis=axis, keepdims=True)
    return (x - m) / jnp.sqrt(v + eps)
def _scatter_add(tgt, idx, src, axis=0):
    return tgt.at[idx].add(src)
def _segment_sum(src, seg, n):
    return jax.ops.segment_sum(src, seg, n)
class _Rng:
    def __init__(self, key):
        self._k = key
    def _next(self):
        self._k, sub = jax.random.split(self._k)
        return sub
    def normal(self, shape):
        return jax.random.normal(self._next(), shape, dtype=jnp.bfloat16)
    def randint(self, lo, hi, shape):
        return jax.random.randint(self._next(), shape, lo, hi, dtype=jnp.int32)
    def uniform(self, shape, lo=0.0, hi=1.0):
        return jax.random.uniform(self._next(), shape, jnp.bfloat16, lo, hi)
    def permutation(self, n):
        return jax.random.permutation(self._next(), n)


kernel_name = 'gated_mix__mha_block__linear_kernel_hedgehog__prompt'

def setup_inputs():
    _rng = _Rng(jax.random.key(int.from_bytes(__import__("os").urandom(4), "little")))
    _w = (lambda a: (lambda t: t.astype(jnp.bfloat16) if jnp.issubdtype(t.dtype, jnp.floating) else t)(jnp.asarray(a)))
    def _A_setup():
        B, S, D, H = 1, 2048, 640, 32
        return {
            "x": _w((lambda *s: _rng.normal(s) * 0.05)(B, S, D)),
            "wqkv": _w((lambda *s: _rng.normal(s) * 0.4)(D, 3 * D)),
            "wo": _w((lambda *s: _rng.normal(s) * 0.05)(D, D)),
        }
    _A_in = _A_setup()

    def _B_setup():
        B, S, D, H = 1, 2048, 640, 32
        Dh = D // H
        return {
            "x": _w((lambda *s: _rng.normal(s) * 0.05)(B, S, D)),
            "wqkv": _w((lambda *s: _rng.normal(s) * 0.8)(D, 3 * D)),
            "w_phi": _w((lambda *s: _rng.normal(s) * 0.8)(H, Dh, Dh) * (Dh ** -0.5)),
            "wo": _w((lambda *s: _rng.normal(s) * 0.05)(D, D)),
        }
    _B_in = _B_setup()

    return {
        "A_x": _A_in["x"],
        "A_wqkv": _A_in["wqkv"],
        "A_wo": _A_in["wo"],
        "B_x": _B_in["x"],
        "B_wqkv": _B_in["wqkv"],
        "B_w_phi": _B_in["w_phi"],
        "B_wo": _B_in["wo"],
        "gate_w": _w((lambda *s: _rng.normal(s) * 0.05)(640) * 16.0),
    }

def reference(A_x, A_wqkv, A_wo, B_x, B_wqkv, B_w_phi, B_wo, gate_w):
    def _A_ref(x, wqkv, wo):
        B, S, D = x.shape
        H = 32
        Dh = D // H
        qkv = (lambda x, *d: x.transpose(*d))((x @ wqkv).reshape(B, S, 3, H, Dh), 2, 0, 3, 1, 4)
        q, k, v = qkv[0], qkv[1], qkv[2]
        scores = jnp.einsum("bhqd,bhkd->bhqk", q, k) * (Dh ** -0.5)
        p = _softmax(scores, axis=-1)
        o = jnp.einsum("bhqk,bhkd->bhqd", p, v)
        return (lambda x, *d: x.transpose(*d))(o, 0, 2, 1, 3).reshape(B, S, D) @ wo

    def _B_ref(x, wqkv, w_phi, wo):
        B, S, D = x.shape
        H = 32; Dh = D // H
        qkv = (lambda x, *d: x.transpose(*d))((x @ wqkv).reshape(B, S, 3, H, Dh), 2, 0, 3, 1, 4)
        q, k, v = qkv[0], qkv[1], qkv[2]
        pq = jnp.einsum("bhsd,hdf->bhsf", q, w_phi)
        pk = jnp.einsum("bhsd,hdf->bhsf", k, w_phi)
        phi_q = jnp.concatenate([_softmax(pq, axis=-1), _softmax(-pq, axis=-1)], axis=-1)
        phi_k = jnp.concatenate([_softmax(pk, axis=-1), _softmax(-pk, axis=-1)], axis=-1)
        kv = jnp.einsum("bhsf,bhsd->bhfd", phi_k, v)
        z  = jnp.einsum("bhsf->bhf", phi_k)
        num = jnp.einsum("bhqf,bhfd->bhqd", phi_q, kv)
        den = jnp.einsum("bhqf,bhf->bhq", phi_q, z)[..., None] + 1e-6
        o = num / den
        return (lambda x, *d: x.transpose(*d))(o, 0, 2, 1, 3).reshape(B, S, D) @ wo

    x = A_x
    g = _sigmoid((x * gate_w).sum(-1, keepdims=True))
    a = _A_ref(x, A_wqkv, A_wo)
    b = _B_ref(x, B_wqkv, B_w_phi, B_wo)
    return g * a + (1 - g) * b
```

```python
import functools, math
import jax
import jax.numpy as jnp
from jax import lax
from jax.experimental import pallas as pl
from jax.experimental.pallas import tpu as pltpu

S = 2048; D = 640; H = 32; DH = 20
TQ = 512; NQ = S // TQ
C = 128; NCH = S // C
L = 1
UPB = 4
NU = NQ * H
VR = 24
F32 = jnp.float32; BF16 = jnp.bfloat16
QSCALE = (DH ** -0.5) * math.log2(math.e)
LOG2E = math.log2(math.e)
NT = (((1,), (1,)), ((), ()))
TP = 512
LTR = 4 * D + 16


def _kernel(x_hbm, wa_hbm, woa_hbm, wb_hbm, wphi_ref, wob_hbm, gate_ref, out_hbm,
            x_v, wa_v, wb_v, woa_v, wob_v,
            wqk, lt, wot, w2, qs, ks, vs, pq_pos, pq_neg, pk_pos, pk_neg, vb, g_row,
            sA, sB, mA, mB, accs, ot, out_v, sems):
    cps = [pltpu.make_async_copy(x_hbm, x_v, sems.at[0]),
           pltpu.make_async_copy(wa_hbm, wa_v, sems.at[1]),
           pltpu.make_async_copy(wb_hbm, wb_v, sems.at[2]),
           pltpu.make_async_copy(woa_hbm, woa_v, sems.at[3]),
           pltpu.make_async_copy(wob_hbm, wob_v, sems.at[4])]
    for cp in cps:
        cp.start()
    for cp in cps:
        cp.wait()

    zpad = jnp.zeros((D, 8), BF16)
    for part in range(2):
        for g in range(6):
            w = min(120, D - 120 * g)
            src = wa_v[:, part * D + 120 * g: part * D + 120 * g + w]
            col = part * 768 + 128 * g
            wqk[:, col: col + w] = src
            wqk[:, col + w: col + 128] = jnp.zeros((D, 128 - w), BF16)
    for h in range(H):
        w2[20 * h: 20 * h + 20, 0:20] = wphi_ref[h].astype(F32)
    w2v = w2[:, 0:20].astype(BF16)
    ei = lax.broadcasted_iota(jnp.int32, (20, D), 0)
    ej = lax.broadcasted_iota(jnp.int32, (20, D), 1)
    E = jnp.where(ej % 20 == ei, 1.0, 0.0).astype(BF16)
    tiled = jnp.dot(w2v, E, preferred_element_type=F32)
    ri = lax.broadcasted_iota(jnp.int32, (D, D), 0) // 20
    ci = lax.broadcasted_iota(jnp.int32, (D, D), 1) // 20
    bd = jnp.where(ri == ci, tiled, 0.0).astype(BF16)
    wq2 = jnp.dot(wb_v[:, 0:D], bd, preferred_element_type=F32) * LOG2E
    wk2 = jnp.dot(wb_v[:, D:2 * D], bd, preferred_element_type=F32) * LOG2E
    lt[0:D, :] = wa_v[:, 2 * D:3 * D].astype(F32).T.astype(BF16)
    lt[D:2 * D, :] = wq2.T.astype(BF16)
    lt[2 * D:3 * D, :] = wk2.T.astype(BF16)
    lt[3 * D:4 * D, :] = wb_v[:, 2 * D:3 * D].astype(F32).T.astype(BF16)
    lt[4 * D:4 * D + 16, :] = jnp.broadcast_to(gate_ref[...], (16, D))
    wot[:, 0:D] = woa_v[...].astype(F32).T.astype(BF16)
    wot[:, D:2 * D] = wob_v[...].astype(F32).T.astype(BF16)

    sub = lax.broadcasted_iota(jnp.int32, (16, 8, TP), 1)
    lo = sub < 4
    NEG = -jnp.inf

    def feat(y, pos_ref, neg_ref, cols):
        y3 = y.reshape(16, 40, TP)
        a = [y3[:, 8 * i: 8 * i + 8, :] for i in range(5)]
        mxE = jnp.max(jnp.maximum(jnp.maximum(a[0], a[1]), jnp.where(lo, a[2], NEG)), axis=1, keepdims=True)
        mxO = jnp.max(jnp.maximum(jnp.maximum(a[3], a[4]), jnp.where(lo, NEG, a[2])), axis=1, keepdims=True)
        mnE = jnp.min(jnp.minimum(jnp.minimum(a[0], a[1]), jnp.where(lo, a[2], -NEG)), axis=1, keepdims=True)
        mnO = jnp.min(jnp.minimum(jnp.minimum(a[3], a[4]), jnp.where(lo, -NEG, a[2])), axis=1, keepdims=True)
        mx = [mxE, mxE, jnp.where(lo, mxE, mxO), mxO, mxO]
        mn = [mnE, mnE, jnp.where(lo, mnE, mnO), mnO, mnO]
        for sign, mm, ref in ((1, mx, pos_ref), (-1, mn, neg_ref)):
            e = [jnp.exp2(a[i] - mm[i]) if sign == 1 else jnp.exp2(mm[i] - a[i]) for i in range(5)]
            sE = jnp.sum(e[0] + e[1] + jnp.where(lo, e[2], 0.0), axis=1, keepdims=True)
            sO = jnp.sum(e[3] + e[4] + jnp.where(lo, 0.0, e[2]), axis=1, keepdims=True)
            rE = 1.0 / sE; rO = 1.0 / sO
            rr = [rE, rE, jnp.where(lo, rE, rO), rO, rO]
            ph = jnp.concatenate([e[i] * rr[i] for i in range(5)], axis=1).reshape(D, TP)
            ref[:, cols] = ph.astype(BF16)

    def proj(tt, carry):
        r0 = pl.multiple_of(tt * TP, TP)
        cols = pl.ds(r0, TP)
        xt = x_v[cols, :]
        qk = jnp.dot(xt, wqk[...], preferred_element_type=F32)
        for g in range(6):
            qs[g, cols, :] = (qk[:, 128 * g: 128 * g + 128] * QSCALE).astype(BF16)
            ks[g, cols, :] = qk[:, 768 + 128 * g: 768 + 128 * g + 128].astype(BF16)
        yt = lax.dot_general(lt[...], xt, NT, preferred_element_type=F32)
        v3 = yt[0:D, :].reshape(16, 40, TP)
        a = [v3[:, 8 * i: 8 * i + 8, :] for i in range(5)]
        e2 = jnp.where(lo, a[2], jnp.where(sub == 4, 1.0, 0.0))
        o0 = jnp.where(lo, jnp.where(sub == 0, 1.0, 0.0), a[2])
        ve = jnp.concatenate([a[0], a[1], e2, o0, a[3], a[4]], axis=1)
        vs[:, :, cols] = ve.reshape(H, VR, TP)
        feat(yt[D:2 * D, :], pq_pos, pq_neg, cols)
        feat(yt[2 * D:3 * D, :], pk_pos, pk_neg, cols)
        vb[:, cols] = yt[3 * D:4 * D, :].astype(BF16)
        z = yt[4 * D:4 * D + 8, :]
        g_row[:, cols] = 1.0 / (1.0 + jnp.exp(-z))
        return carry
    lax.fori_loop(0, S // TP, proj, 0)

    rr = lax.broadcasted_iota(jnp.int32, (96, 80), 0)
    cc = lax.broadcasted_iota(jnp.int32, (96, 80), 1) // 20
    hrow = jnp.where(rr < 80, rr // 20, rr - 80)
    bmask = hrow == cc
    ones_blk = jnp.where(lax.broadcasted_iota(jnp.int32, (16, S), 0) < 4, 1.0, 0.0).astype(BF16)
    sub2 = lax.broadcasted_iota(jnp.int32, (8, S), 0)
    lo2 = sub2 < 4
    gB = 1.0 - g_row[0:1, :]
    for G in range(8):
        rows = slice(80 * G, 80 * G + 80)
        vext = jnp.concatenate([vb[rows, :], ones_blk], axis=0)
        kvp = lax.dot_general(vext, pk_pos[rows, :], NT, preferred_element_type=F32)
        kvn = lax.dot_general(vext, pk_neg[rows, :], NT, preferred_element_type=F32)
        kvp = jnp.where(bmask, kvp, 0.0).astype(BF16)
        kvn = jnp.where(bmask, kvn, 0.0).astype(BF16)
        nd = (jnp.dot(kvp, pq_pos[rows, :], preferred_element_type=F32)
              + jnp.dot(kvn, pq_neg[rows, :], preferred_element_type=F32))
        rden = gB / (nd[80:88, :] + 1e-6)
        for p in range(2):
            rE = rden[2 * p: 2 * p + 1, :]; rO = rden[2 * p + 1: 2 * p + 2, :]
            b0 = 40 * p
            ot[D + 80 * G + b0: D + 80 * G + b0 + 16, :] = nd[b0: b0 + 16, :] * rE
            ot[D + 80 * G + b0 + 16: D + 80 * G + b0 + 24, :] = nd[b0 + 16: b0 + 24, :] * jnp.where(lo2, rE, rO)
            ot[D + 80 * G + b0 + 24: D + 80 * G + b0 + 40, :] = nd[b0 + 24: b0 + 40, :] * rO

    lane = lax.broadcasted_iota(jnp.int32, (TQ, 128), 1)
    lo3 = lax.broadcasted_iota(jnp.int32, (8, TQ), 0) < 4

    def get_qm(u):
        t = u // H; h = u % H
        g = h // 6; off = (h % 6) * 20
        q = qs[g, pl.ds(pl.multiple_of(t * TQ, TQ), TQ), :]
        return g, jnp.where((lane >= off) & (lane < off + 20), q, jnp.zeros_like(q))

    def s1_chunk(c, g, qm, s_ref, m8):
        k = ks[g, c * C:(c + 1) * C, :]
        s = lax.dot_general(k, qm, NT, preferred_element_type=F32)
        s_ref[c * C:(c + 1) * C, :] = s
        mm = jnp.max(s.reshape(C // 8, 8, TQ), axis=0)
        return mm if m8 is None else jnp.maximum(m8, mm)

    def s2_chunk(c, h, m, s_ref, acc):
        p = jnp.exp2(s_ref[c * C:(c + 1) * C, :] - m)
        v = vs[h, :, c * C:(c + 1) * C]
        r = jnp.dot(v, p, preferred_element_type=F32)
        return r if acc is None else acc + r

    def fin(u, acc, odd):
        t = u // H; h = u % H
        cols = pl.ds(pl.multiple_of(t * TQ, TQ), TQ)
        g = g_row[0:1, cols]
        base = pl.multiple_of((h // 2) * 40, 8)
        if not odd:
            r = g / acc[20:21, :]
            ot[pl.ds(base, 16), cols] = acc[0:16, :] * r
            accs_even[...] = acc[16:24, :] * r
        else:
            r = g / acc[0:1, :]
            ot[pl.ds(base + 16, 8), cols] = jnp.where(lo3, accs_even[...], acc[0:8, :] * r)
            ot[pl.ds(base + 24, 16), cols] = acc[8:24, :] * r

    accs_acc = accs.at[0:VR, :]
    accs_even = accs.at[VR:VR + 8, :]

    def unit(u, s_nxt, m_nxt, s_cur, m_cur, acc_prev, odd):
        u1 = jnp.minimum(u + 1, NU - 1)
        g, qm = get_qm(u1)
        mprev = m_nxt[0:1, :]
        m = m_cur[0:1, :]
        m8 = None; acc = None
        up = jnp.maximum(u - 1, 0)
        for i in range(NCH):
            if i < L:
                acc_prev = s2_chunk(NCH - L + i, up % H, mprev, s_nxt, acc_prev)
                m8 = s1_chunk(i, g, qm, s_nxt, m8)
                if i == L - 1:
                    fin(up, acc_prev, not odd)
            else:
                m8 = s1_chunk(i, g, qm, s_nxt, m8)
                acc = s2_chunk(i - L, u % H, m, s_cur, acc)
        m_nxt[...] = jnp.broadcast_to(jnp.max(m8, axis=0, keepdims=True), (8, TQ))
        return acc

    g0, qm0 = get_qm(0)
    m8 = None
    for c in range(NCH):
        m8 = s1_chunk(c, g0, qm0, sA, m8)
    mA[...] = jnp.broadcast_to(jnp.max(m8, axis=0, keepdims=True), (8, TQ))
    sB[...] = jnp.zeros_like(sB)
    mB[...] = jnp.zeros_like(mB)
    accs[...] = jnp.ones_like(accs)

    def body(j, carry):
        acc = accs_acc[...]
        for r in range(UPB):
            u = UPB * j + r
            if r % 2 == 0:
                acc = unit(u, sB, mB, sA, mA, acc, False)
            else:
                acc = unit(u, sA, mA, sB, mB, acc, True)
        accs_acc[...] = acc
        return carry
    lax.fori_loop(0, NU // UPB, body, 0)
    acc = accs_acc[...]
    m = mB[0:1, :]
    for i in range(L):
        acc = s2_chunk(NCH - L + i, (NU - 1) % H, m, sB, acc)
    fin(NU - 1, acc, True)

    def outp(t, carry):
        cols = pl.ds(pl.multiple_of(t * TQ, TQ), TQ)
        o = ot[:, cols].astype(BF16)
        yT = jnp.dot(wot[...], o, preferred_element_type=F32)
        out_v[cols, :] = yT.T.astype(BF16)
        return carry
    lax.fori_loop(0, NQ, outp, 0)
    cp = pltpu.make_async_copy(out_v, out_hbm, sems.at[5])
    cp.start(); cp.wait()


@jax.jit
def pallas_gated_mix__mha_block__linear_kernel_hedgehog__prompt_kernel(A_x, A_wqkv, A_wo, B_x, B_wqkv, B_w_phi, B_wo, gate_w):
    x = A_x.reshape(S, D)
    gate = gate_w.reshape(1, D)
    any_spec = pl.BlockSpec(memory_space=pl.ANY)
    vm = pl.BlockSpec(memory_space=pltpu.VMEM)
    out = pl.pallas_call(
        _kernel,
        out_shape=jax.ShapeDtypeStruct((S, D), BF16),
        in_specs=[any_spec, any_spec, any_spec, any_spec, vm, any_spec, vm],
        out_specs=any_spec,
        scratch_shapes=[
            pltpu.VMEM((S, D), BF16), pltpu.VMEM((D, 3 * D), BF16), pltpu.VMEM((D, 3 * D), BF16),
            pltpu.VMEM((D, D), BF16), pltpu.VMEM((D, D), BF16),
            pltpu.VMEM((D, 1536), BF16), pltpu.VMEM((LTR, D), BF16), pltpu.VMEM((D, 2 * D), BF16),
            pltpu.VMEM((D, 128), F32),
            pltpu.VMEM((6, S, 128), BF16), pltpu.VMEM((6, S, 128), BF16), pltpu.VMEM((H, VR, S), F32),
            pltpu.VMEM((D, S), BF16), pltpu.VMEM((D, S), BF16), pltpu.VMEM((D, S), BF16), pltpu.VMEM((D, S), BF16),
            pltpu.VMEM((D, S), BF16), pltpu.VMEM((8, S), F32),
            pltpu.VMEM((S, TQ), F32), pltpu.VMEM((S, TQ), F32),
            pltpu.VMEM((8, TQ), F32), pltpu.VMEM((8, TQ), F32), pltpu.VMEM((VR + 8, TQ), F32),
            pltpu.VMEM((2 * D, S), F32), pltpu.VMEM((S, D), BF16),
            pltpu.SemaphoreType.DMA((6,)),
        ],
        compiler_params=pltpu.CompilerParams(vmem_limit_bytes=110 * 1024 * 1024),
    )(x, A_wqkv, A_wo, B_wqkv, B_w_phi, B_wo, gate)
    return out.reshape(1, S, D)
```

```python
import math
import jax
import jax.numpy as jnp
from jax import lax
from jax.experimental import pallas as pl
from jax.experimental.pallas import tpu as pltpu

S = 2048; D = 640; H = 32; DH = 20
TQ = 512; NQ = S // TQ
C = 128; NCH = S // C
L = 1
UPB = 8
UPB_SLOW = 2
NU = NQ * H
VR = 24
F32 = jnp.float32; BF16 = jnp.bfloat16
LOG2E = math.log2(math.e)
QSCALE = (DH ** -0.5) * LOG2E
BOUND_MAX = 30.0
NT = (((1,), (1,)), ((), ()))
TP = 512
LTR = 5 * D + 16
BAND = [((80 * G) // 128, (80 * G + 79) // 128 + 1) for G in range(8)]
BROW = 120


def _kernel(x_hbm, wa_hbm, woa_hbm, wb_hbm, wphi_ref, wob_hbm, gate_ref, out_hbm,
            x_v, wak_v, waq_v, wav_v, wb_v, wo_v,
            wkt, lt, mscr, tbd, qt, ks, vs, pq_pos, pq_neg, pk_pos, pk_neg, vb, g_row,
            kn, nb, bmx,
            sA, accs, qm0, qm1, qm2, qm3, s0, ot, out_v, sems, osems):
    cp_wk = pltpu.make_async_copy(wa_hbm.at[:, D:2 * D], wak_v, sems.at[0])
    cp_x = [pltpu.make_async_copy(x_hbm.at[pl.ds(i * TP, TP), :], x_v.at[pl.ds(i * TP, TP), :], sems.at[1 + i])
            for i in range(4)]
    cp_wq = pltpu.make_async_copy(wa_hbm.at[:, 0:D], waq_v, sems.at[9])
    cp_wav = pltpu.make_async_copy(wa_hbm.at[:, 2 * D:3 * D], wav_v, sems.at[5])
    cp_wb = pltpu.make_async_copy(wb_hbm, wb_v, sems.at[6])
    cp_woa = pltpu.make_async_copy(woa_hbm, wo_v.at[0:D, :], sems.at[7])
    cp_wob = pltpu.make_async_copy(wob_hbm, wo_v.at[D:2 * D, :], sems.at[8])
    cp_wk.start()
    cp_x[0].start()

    for d in range(DH):
        mscr[0:DH, 32 * d: 32 * d + 32] = wphi_ref[d].astype(F32)
    m1 = mscr[0:DH, :].astype(BF16)
    pi = lax.broadcasted_iota(jnp.int32, (D, D), 0)
    pj = lax.broadcasted_iota(jnp.int32, (D, D), 1)
    perm = jnp.where(pj == 20 * (pi & 31) + (pi >> 5), 1.0, 0.0).astype(BF16)
    m2 = jnp.dot(m1, perm, preferred_element_type=F32).astype(BF16)
    ei = lax.broadcasted_iota(jnp.int32, (D, DH), 0)
    ej = lax.broadcasted_iota(jnp.int32, (D, DH), 1)
    et = jnp.where(((ei - 80 * ((ei * 3277) >> 18)) >> 2) == ej, 1.0, 0.0).astype(BF16)
    tiled = jnp.dot(et, m2, preferred_element_type=F32)
    same = (4 * ((pi * 3277) >> 18) + (pi & 3)) == ((pj * 3277) >> 16)
    tbd[...] = jnp.where(same, tiled, 0.0).astype(BF16)

    for cp in cp_x[1:]:
        cp.start()
    cp_wq.start(); cp_wav.start(); cp_wb.start(); cp_woa.start(); cp_wob.start()

    sub = lax.broadcasted_iota(jnp.int32, (16, 8, TP), 1)
    lo = sub < 4

    def tr(w):
        return w.astype(F32).T.astype(BF16)

    def slabs(y):
        y3 = y.reshape(16, 40, TP)
        return [y3[:, 8 * i: 8 * i + 8, :] for i in range(5)]

    def pairnorm(y):
        y3 = y.reshape(16, 40, TP)
        return jnp.sum(y3 * y3, axis=1, keepdims=True)

    def rev8(a):
        n = a.shape[0]
        return jnp.concatenate([a[128 * b + 8 * (15 - j): 128 * b + 8 * (15 - j) + 8, :]
                                for b in range(n // 128) for j in range(16)], axis=0)

    def k_proj(tt):
        rows = pl.ds(tt * TP if isinstance(tt, int) else pl.multiple_of(tt * TP, TP), TP)
        kt = lax.dot_general(wkt[...], x_v[rows, :], NT, preferred_element_type=F32)
        for g in range(6):
            w = min(120, D - 120 * g)
            parts = [kt[120 * g: 120 * g + w, :]]
            if w < BROW:
                parts.append(jnp.zeros((BROW - w, TP), F32))
            parts.append(jnp.where(lax.broadcasted_iota(jnp.int32, (8, TP), 0) == 0, 1.0, 0.0))
            ks[g, rows, :] = rev8(jnp.concatenate(parts, axis=0).T).astype(BF16)
        n = jnp.broadcast_to(pairnorm(kt), (16, 8, TP))
        kn[...] = n if isinstance(tt, int) and tt == 0 else jnp.maximum(kn[...], n)

    def fold(off, row0):
        for j, (k0, k1) in enumerate(BAND):
            r = lax.dot_general(tbd[80 * j: 80 * j + 80, 128 * k0: 128 * k1],
                                wb_v[:, off + 128 * k0: off + 128 * k1], NT, preferred_element_type=F32)
            lt[row0 + 80 * j: row0 + 80 * j + 80, :] = (r * LOG2E).astype(BF16)

    cp_wk.wait()
    wkt[...] = tr(wak_v[...])
    cp_x[0].wait()
    k_proj(0)
    cp_x[1].wait(); cp_x[2].wait()
    if True:
        lax.fori_loop(1, 3, lambda tt, c: (k_proj(tt), c)[1], 0)
    else:
        k_proj(1)
        k_proj(2)
    cp_x[3].wait(); cp_wq.wait(); cp_wav.wait()
    lt[4 * D:5 * D, :] = tr(waq_v[...])
    k_proj(3)
    lt[0:D, :] = tr(wav_v[...])
    cp_wb.wait()
    fold(0, D)
    lt[3 * D:4 * D, :] = tr(wb_v[:, 2 * D:3 * D])
    fold(D, 2 * D)
    lt[5 * D:5 * D + 16, :] = jnp.broadcast_to(gate_ref[...].astype(F32).reshape(1, D), (16, D)).astype(BF16)
    for g in range(6):
        w = min(120, D - 120 * g)
        qt[g, w:128, :] = jnp.zeros((128 - w, S), BF16)
    kn[...] = jnp.broadcast_to(jnp.max(kn[...], axis=2, keepdims=True), (16, 8, TP))
    bmx[...] = jnp.zeros_like(bmx)

    def feat(y, pos_ref, neg_ref, cols):
        y4 = y.reshape(8, 10, 8, TP)
        mx = jnp.max(y4, axis=1); mx = jnp.maximum(mx, pltpu.roll(mx, 4, 1))[:, None]
        mn = jnp.min(y4, axis=1); mn = jnp.minimum(mn, pltpu.roll(mn, 4, 1))[:, None]
        for e, ref in ((jnp.exp2(y4 - mx), pos_ref), (jnp.exp2(mn - y4), neg_ref)):
            s = jnp.sum(e, axis=1); s = s + pltpu.roll(s, 4, 1)
            ref[:, cols] = (e * (1.0 / s)[:, None]).reshape(D, TP).astype(BF16)

    def proj(tt, carry):
        r0 = pl.multiple_of(tt * TP, TP)
        cols = pl.ds(r0, TP)
        yt = lax.dot_general(lt[...], x_v[cols, :], NT, preferred_element_type=F32)
        a = slabs(yt[0:D, :])
        e2 = jnp.where(lo, a[2], jnp.where(sub == 4, 1.0, 0.0))
        o0 = jnp.where(lo, jnp.where(sub == 0, 1.0, 0.0), a[2])
        ve = jnp.concatenate([a[0], a[1], e2, o0, a[3], a[4]], axis=1)
        vs[:, :, cols] = ve.reshape(H, VR, TP)
        feat(yt[D:2 * D, :], pq_pos, pq_neg, cols)
        feat(yt[2 * D:3 * D, :], pk_pos, pk_neg, cols)
        vb[:, cols] = yt[3 * D:4 * D, :].astype(BF16)
        q = yt[4 * D:5 * D, :] * QSCALE
        for g in range(6):
            w = min(120, D - 120 * g)
            qt[g, 0:w, cols] = q[120 * g: 120 * g + w, :].astype(BF16)
        bnd = jnp.sqrt(pairnorm(q) * kn[...])
        nb[:, :, cols] = -bnd
        bmx[...] = jnp.maximum(bmx[...], bnd)
        z = yt[5 * D:5 * D + 8, :]
        g_row[:, cols] = 1.0 / (1.0 + jnp.exp(-z))
        return carry
    lax.fori_loop(0, S // TP, proj, 0)

    cp_woa.wait()
    cp_wob.wait()
    rr = lax.broadcasted_iota(jnp.int32, (96, 80), 0)
    cc = lax.broadcasted_iota(jnp.int32, (96, 80), 1) & 3
    hrow = jnp.where(rr < 80, (rr * 3277) >> 16, rr - 80)
    bmask = hrow == cc
    lo2 = lax.broadcasted_iota(jnp.int32, (8, S), 0) < 4

    def al8(v):
        return v if isinstance(v, int) else pl.multiple_of(v, 8)

    def bmid(G, carry):
        r0 = 80 * G if isinstance(G, int) else pl.multiple_of(80 * G, 16)
        rows = pl.ds(r0, 80)
        ones_blk = jnp.where(lax.broadcasted_iota(jnp.int32, (16, S), 0) < 4, 1.0, 0.0).astype(BF16)
        vext = jnp.concatenate([vb[rows, :], ones_blk], axis=0)
        kvp = lax.dot_general(vext, pk_pos[rows, :], NT, preferred_element_type=F32)
        kvn = lax.dot_general(vext, pk_neg[rows, :], NT, preferred_element_type=F32)
        kvp = jnp.where(bmask, kvp, 0.0).astype(BF16)
        kvn = jnp.where(bmask, kvn, 0.0).astype(BF16)
        nd = (jnp.dot(kvp, pq_pos[rows, :], preferred_element_type=F32)
              + jnp.dot(kvn, pq_neg[rows, :], preferred_element_type=F32))
        rden = (1.0 - g_row[0:1, :]) / (nd[80:88, :] + 1e-6)
        for p in range(2):
            rE = rden[2 * p: 2 * p + 1, :]; rO = rden[2 * p + 1: 2 * p + 2, :]
            b0 = 40 * p
            o0 = D + r0 + b0
            ot[pl.ds(al8(o0), 16), :] = nd[b0: b0 + 16, :] * rE
            ot[pl.ds(al8(o0 + 16), 8), :] = nd[b0 + 16: b0 + 24, :] * jnp.where(lo2, rE, rO)
            ot[pl.ds(al8(o0 + 24), 16), :] = nd[b0 + 24: b0 + 40, :] * rO
        return carry
    BU = 8
    if BU == 8:
        for G in range(8):
            bmid(G, 0)
    else:
        def bloop(j, c):
            for r in range(BU):
                bmid(BU * j + r, 0)
            return c
        lax.fori_loop(0, 8 // BU, bloop, 0)

    row16 = lax.broadcasted_iota(jnp.int32, (16, TQ), 0)
    lo3 = lax.broadcasted_iota(jnp.int32, (8, TQ), 0) < 4
    accs_even = accs.at[VR:VR + 8, :]

    def grp(u):
        return ((u & 31) * 43) >> 8

    def prep_qm(u, qm_ref, shift, piece=None):
        t = u >> 5; h = u & 31
        g = grp(u); off = (h - 6 * g) * 20
        cols = pl.ds(pl.multiple_of(t * TQ, TQ), TQ)
        for i in (range(8) if piece is None else (piece,)):
            q = qt[g, 16 * i: 16 * i + 16, cols]
            row = row16 + 16 * i
            qm = jnp.where((row >= off) & (row < off + 20), q, jnp.zeros_like(q))
            if shift and i == BROW // 16:
                b = nb[h >> 1, :, cols]
                qm = jnp.where(row == BROW, jnp.concatenate([b, b], axis=0).astype(BF16), qm)
            qm_ref[16 * i: 16 * i + 16, :] = qm

    def qk_chunk(c, g, qm_ref):
        return jnp.dot(ks[g, c * C:(c + 1) * C, :], qm_ref[...], preferred_element_type=F32)

    def pv_chunk(c, h, p, acc):
        r = jnp.dot(vs[h, :, c * C:(c + 1) * C], rev8(p), preferred_element_type=F32)
        return r if acc is None else acc + r

    def fin(u, acc, odd):
        t = u >> 5; h = u & 31
        cols = pl.ds(pl.multiple_of(t * TQ, TQ), TQ)
        g = g_row[0:1, cols]
        base = pl.multiple_of((h >> 1) * 40, 8)
        if not odd:
            r = g / acc[20:21, :]
            ot[pl.ds(base, 16), cols] = acc[0:16, :] * r
            accs_even[...] = acc[16:24, :] * r
        else:
            r = g / acc[0:1, :]
            ot[pl.ds(base + 16, 8), cols] = jnp.where(lo3, accs_even[...], acc[0:8, :] * r)
            ot[pl.ds(base + 24, 16), cols] = acc[8:24, :] * r

    safe = jnp.max(bmx[...]) <= BOUND_MAX

    @pl.when(safe)
    def _fast():
        qms = (qm0, qm1, qm2, qm3)
        prep_qm(0, qm0, True)
        prep_qm(1, qm1, True)
        s0[...] = qk_chunk(0, 0, qm0)

        def body(j, carry):
            s = s0[...]
            for r in range(UPB):
                u = UPB * j + r
                odd = r % 2 == 1
                qm_cur, qm_nxt, qm_prep = qms[r % 4], qms[(r + 1) % 4], qms[(r + 2) % 4]
                u1 = jnp.minimum(u + 1, NU - 1)
                u2 = jnp.minimum(u + 2, NU - 1)
                g = grp(u); g1 = grp(u1)
                acc = None
                for c in range(NCH):
                    if c + 1 < NCH:
                        s_next = qk_chunk(c + 1, g, qm_cur)
                    else:
                        s_next = qk_chunk(0, g1, qm_nxt)
                    acc = pv_chunk(c, u & 31, jnp.exp2(s), acc)
                    s = s_next
                    if 4 <= c < 12:
                        prep_qm(u2, qm_prep, True, c - 4)
                fin(u, acc, odd)
            s0[...] = s
            return carry
        lax.fori_loop(0, NU // UPB, body, 0)

    @pl.when(jnp.logical_not(safe))
    def _slow():
        def unit(u, odd):
            g = grp(u); h = u & 31
            prep_qm(u, qm0, False)

            def p1(c, m8):
                r0 = pl.multiple_of(c * C, C)
                s = jnp.dot(ks[g, pl.ds(r0, C), :], qm0[...], preferred_element_type=F32)
                sA[pl.ds(r0, C), :] = s
                return jnp.maximum(m8, jnp.max(s.reshape(C // 8, 8, TQ), axis=0))
            m8 = lax.fori_loop(0, NCH, p1, jnp.full((8, TQ), -jnp.inf, F32))
            m = jnp.max(m8, axis=0, keepdims=True)

            def p2(c, acc):
                r0 = pl.multiple_of(c * C, C)
                p = jnp.exp2(sA[pl.ds(r0, C), :] - m)
                return acc + jnp.dot(vs[h, :, pl.ds(r0, C)], rev8(p), preferred_element_type=F32)
            acc = lax.fori_loop(0, NCH, p2, jnp.zeros((VR, TQ), F32))
            fin(u, acc, odd)

        def body(j, carry):
            unit(2 * j, False)
            unit(2 * j + 1, True)
            return carry
        lax.fori_loop(0, NU // 2, body, 0)

    OPB = 1
    def outp(j, carry):
        for r in range(OPB):
            t = OPB * j + r
            cols = pl.ds(pl.multiple_of(t * TQ, TQ), TQ)
            o = ot[:, cols].astype(BF16)
            y = lax.dot_general(o, wo_v[...], (((0,), (0,)), ((), ())), preferred_element_type=F32)
            out_v[cols, :] = y.astype(BF16)
            pltpu.make_async_copy(out_v.at[cols, :], out_hbm.at[cols, :], osems.at[t]).start()
        return carry
    lax.fori_loop(0, NQ // OPB, outp, 0)
    for t in range(NQ):
        rows = pl.ds(t * TQ, TQ)
        pltpu.make_async_copy(out_v.at[rows, :], out_hbm.at[rows, :], osems.at[t]).wait()


@jax.jit
def pallas_gated_mix__mha_block__linear_kernel_hedgehog__prompt_kernel(A_x, A_wqkv, A_wo, B_x, B_wqkv, B_w_phi, B_wo, gate_w):
    x = A_x.reshape(S, D)
    wphi = jnp.transpose(B_w_phi, (1, 2, 0))
    any_spec = pl.BlockSpec(memory_space=pl.ANY)
    vm = pl.BlockSpec(memory_space=pltpu.VMEM)
    out = pl.pallas_call(
        _kernel,
        out_shape=jax.ShapeDtypeStruct((S, D), BF16),
        in_specs=[any_spec, any_spec, any_spec, any_spec, vm, any_spec, vm],
        out_specs=any_spec,
        scratch_shapes=[
            pltpu.VMEM((S, D), BF16), pltpu.VMEM((D, D), BF16), pltpu.VMEM((D, D), BF16), pltpu.VMEM((D, D), BF16),
            pltpu.VMEM((D, 3 * D), BF16), pltpu.VMEM((2 * D, D), BF16),
            pltpu.VMEM((D, D), BF16), pltpu.VMEM((LTR, D), BF16),
            pltpu.VMEM((24, D), F32), pltpu.VMEM((D, D), BF16),
            pltpu.VMEM((6, 128, S), BF16), pltpu.VMEM((6, S, 128), BF16), pltpu.VMEM((H, VR, S), F32),
            pltpu.VMEM((D, S), BF16), pltpu.VMEM((D, S), BF16), pltpu.VMEM((D, S), BF16), pltpu.VMEM((D, S), BF16),
            pltpu.VMEM((D, S), BF16), pltpu.VMEM((8, S), F32),
            pltpu.VMEM((16, 8, TP), F32), pltpu.VMEM((16, 8, S), F32), pltpu.VMEM((16, 8, TP), F32),
            pltpu.VMEM((S, TQ), F32), pltpu.VMEM((VR + 8, TQ), F32),
            pltpu.VMEM((128, TQ), BF16), pltpu.VMEM((128, TQ), BF16), pltpu.VMEM((128, TQ), BF16), pltpu.VMEM((128, TQ), BF16), pltpu.VMEM((C, TQ), F32),
            pltpu.VMEM((2 * D, S), F32), pltpu.VMEM((S, D), BF16),
            pltpu.SemaphoreType.DMA((10,)), pltpu.SemaphoreType.DMA((NQ,)),
        ],
        compiler_params=pltpu.CompilerParams(vmem_limit_bytes=110 * 1024 * 1024),
    )(x, A_wqkv, A_wo, B_wqkv, wphi, B_wo, gate_w)
    return out.reshape(1, S, D)
```

```python
import math

import jax
import jax.numpy as jnp
from jax import lax
from jax.experimental import pallas as pl
from jax.experimental.pallas import tpu as pltpu

S = 2048; D = 640; H = 32; DH = 20
TQ = 512; NQ = S // TQ
C = 128; NCH = S // C
UPB = 8
NU = NQ * H
VR = 24
F32 = jnp.float32; BF16 = jnp.bfloat16
LOG2E = math.log2(math.e)
QSCALE = (DH ** -0.5) * LOG2E
BOUND_MAX = 30.0
NT = (((1,), (1,)), ((), ()))
TN = (((0,), (0,)), ((), ()))
TP = 512
LTR = 5 * D + 16
BAND = [((80 * G) // 128, (80 * G + 79) // 128 + 1) for G in range(8)]
BROW = 120


def _kernel(x_hbm, wa_hbm, woa_hbm, wb_hbm, wphi_hbm, wob_hbm, gate_hbm, out_hbm,
            wphi_ref, gate_ref, x_v, wak_v, waq_v, wav_v, wb_v, wo_v,
            wkt, lt, mscr, tbd, qt, ks, vs, pq_pos, pq_neg, pk_pos, pk_neg, vb, g_row,
            kn, nb, bmx,
            sA, a_even, qm0, qm1, qm2, qm3, s0, ot, out_v, sems, osems):
    cp_wk = pltpu.make_async_copy(wa_hbm.at[:, D:2 * D], wak_v, sems.at[0])
    cp_x = [pltpu.make_async_copy(x_hbm.at[pl.ds(i * TP, TP), :], x_v.at[pl.ds(i * TP, TP), :], sems.at[1 + i])
            for i in range(4)]
    cp_wq = pltpu.make_async_copy(wa_hbm.at[:, 0:D], waq_v, sems.at[9])
    cp_wav = pltpu.make_async_copy(wa_hbm.at[:, 2 * D:3 * D], wav_v, sems.at[5])
    cp_wb = pltpu.make_async_copy(wb_hbm, wb_v, sems.at[6])
    cp_woa = pltpu.make_async_copy(woa_hbm, wo_v.at[0:D, :], sems.at[7])
    cp_wob = pltpu.make_async_copy(wob_hbm, wo_v.at[D:2 * D, :], sems.at[8])
    cp_phi = pltpu.make_async_copy(wphi_hbm, wphi_ref, sems.at[10])
    cp_gate = pltpu.make_async_copy(gate_hbm, gate_ref, sems.at[11])
    cp_phi.start()
    cp_wk.start()
    cp_x[0].start()
    cp_gate.start()
    cp_phi.wait()

    for d in range(DH):
        mscr[0:DH, 32 * d: 32 * d + 32] = wphi_ref[d].astype(F32)
    m1 = mscr[0:DH, :].astype(BF16)
    pi = lax.broadcasted_iota(jnp.int32, (D, D), 0)
    pj = lax.broadcasted_iota(jnp.int32, (D, D), 1)
    perm = jnp.where(pj == 20 * (pi & 31) + (pi >> 5), 1.0, 0.0).astype(BF16)
    m2 = jnp.dot(m1, perm, preferred_element_type=F32).astype(BF16)
    ei = lax.broadcasted_iota(jnp.int32, (D, DH), 0)
    ej = lax.broadcasted_iota(jnp.int32, (D, DH), 1)
    et = jnp.where(((ei - 80 * ((ei * 3277) >> 18)) >> 2) == ej, 1.0, 0.0).astype(BF16)
    tiled = jnp.dot(et, m2, preferred_element_type=F32)
    same = (4 * ((pi * 3277) >> 18) + (pi & 3)) == ((pj * 3277) >> 16)
    tbd[...] = jnp.where(same, tiled, 0.0).astype(BF16)

    for cp in cp_x[1:]:
        cp.start()
    cp_wq.start(); cp_wav.start(); cp_wb.start(); cp_woa.start(); cp_wob.start()

    sub = lax.broadcasted_iota(jnp.int32, (16, 8, TP), 1)
    lo = sub < 4

    def tr(w):
        return w.astype(F32).T.astype(BF16)

    def pairnorm(y):
        y3 = y.reshape(16, 40, TP)
        return jnp.sum(y3 * y3, axis=1, keepdims=True)

    def rev8(a):
        n = a.shape[0]
        return jnp.concatenate([a[128 * b + 8 * (15 - j): 128 * b + 8 * (15 - j) + 8, :]
                                for b in range(n // 128) for j in range(16)], axis=0)

    def k_proj(tt):
        rows = pl.ds(tt * TP if isinstance(tt, int) else pl.multiple_of(tt * TP, TP), TP)
        kt = lax.dot_general(wkt[...], x_v[rows, :], NT, preferred_element_type=F32)
        for g in range(6):
            w = min(120, D - 120 * g)
            parts = [kt[120 * g: 120 * g + w, :]]
            if w < BROW:
                parts.append(jnp.zeros((BROW - w, TP), F32))
            parts.append(jnp.where(lax.broadcasted_iota(jnp.int32, (8, TP), 0) == 0, 1.0, 0.0))
            ks[g, rows, :] = rev8(jnp.concatenate(parts, axis=0).T).astype(BF16)
        n = jnp.broadcast_to(pairnorm(kt), (16, 8, TP))
        kn[...] = n if isinstance(tt, int) and tt == 0 else jnp.maximum(kn[...], n)

    def fold(off, row0):
        for j, (k0, k1) in enumerate(BAND):
            r = lax.dot_general(tbd[80 * j: 80 * j + 80, 128 * k0: 128 * k1],
                                wb_v[:, off + 128 * k0: off + 128 * k1], NT, preferred_element_type=F32)
            lt[row0 + 80 * j: row0 + 80 * j + 80, :] = (r * LOG2E).astype(BF16)

    cp_wk.wait()
    wkt[...] = tr(wak_v[...])
    cp_x[0].wait()
    k_proj(0)
    cp_x[1].wait(); cp_x[2].wait()
    lax.fori_loop(1, 3, lambda tt, c: (k_proj(tt), c)[1], 0)
    cp_x[3].wait(); cp_wq.wait(); cp_wav.wait()
    lt[4 * D:5 * D, :] = tr(waq_v[...])
    k_proj(3)
    lt[0:D, :] = tr(wav_v[...])
    cp_wb.wait(); cp_gate.wait()
    fold(0, D)
    lt[3 * D:4 * D, :] = tr(wb_v[:, 2 * D:3 * D])
    fold(D, 2 * D)
    lt[5 * D:5 * D + 16, :] = jnp.broadcast_to(gate_ref[...].astype(F32).reshape(1, D), (16, D)).astype(BF16)
    for g in range(6):
        w = min(120, D - 120 * g)
        qt[g, w:128, :] = jnp.zeros((128 - w, S), BF16)
    kn[...] = jnp.broadcast_to(jnp.max(kn[...], axis=2, keepdims=True), (16, 8, TP))
    bmx[...] = jnp.zeros_like(bmx)

    def feat(y, pos_ref, neg_ref, cols):
        y4 = y.reshape(8, 10, 8, TP)
        mx = jnp.max(y4, axis=1); mx = jnp.maximum(mx, pltpu.roll(mx, 4, 1))[:, None]
        mn = jnp.min(y4, axis=1); mn = jnp.minimum(mn, pltpu.roll(mn, 4, 1))[:, None]
        for e, ref in ((jnp.exp2(y4 - mx), pos_ref), (jnp.exp2(mn - y4), neg_ref)):
            s = jnp.sum(e, axis=1); s = s + pltpu.roll(s, 4, 1)
            ref[:, cols] = (e * (1.0 / s)[:, None]).reshape(D, TP).astype(BF16)

    def proj(tt, carry):
        cols = pl.ds(pl.multiple_of(tt * TP, TP), TP)
        yt = lax.dot_general(lt[...], x_v[cols, :], NT, preferred_element_type=F32)
        v3 = yt[0:D, :].reshape(16, 40, TP)
        a = [v3[:, 8 * i: 8 * i + 8, :] for i in range(5)]
        e2 = jnp.where(lo, a[2], jnp.where(sub == 4, 1.0, 0.0))
        o0 = jnp.where(lo, jnp.where(sub == 0, 1.0, 0.0), a[2])
        ve = jnp.concatenate([a[0], a[1], e2, o0, a[3], a[4]], axis=1)
        vs[:, :, cols] = ve.reshape(H, VR, TP)
        feat(yt[D:2 * D, :], pq_pos, pq_neg, cols)
        feat(yt[2 * D:3 * D, :], pk_pos, pk_neg, cols)
        vb[:, cols] = yt[3 * D:4 * D, :].astype(BF16)
        q = yt[4 * D:5 * D, :] * QSCALE
        for g in range(6):
            w = min(120, D - 120 * g)
            qt[g, 0:w, cols] = q[120 * g: 120 * g + w, :].astype(BF16)
        bnd = jnp.sqrt(pairnorm(q) * kn[...])
        nb[:, :, cols] = -bnd
        bmx[...] = jnp.maximum(bmx[...], bnd)
        z = yt[5 * D:5 * D + 8, :]
        g_row[:, cols] = 1.0 / (1.0 + jnp.exp(-z))
        return carry
    lax.fori_loop(0, S // TP, proj, 0)

    cp_woa.wait()
    cp_wob.wait()
    rr = lax.broadcasted_iota(jnp.int32, (96, 80), 0)
    cc = lax.broadcasted_iota(jnp.int32, (96, 80), 1) & 3
    hrow = jnp.where(rr < 80, (rr * 3277) >> 16, rr - 80)
    bmask = hrow == cc
    lo2 = lax.broadcasted_iota(jnp.int32, (8, S), 0) < 4
    for G in range(8):
        rows = pl.ds(80 * G, 80)
        ones_blk = jnp.where(lax.broadcasted_iota(jnp.int32, (16, S), 0) < 4, 1.0, 0.0).astype(BF16)
        vext = jnp.concatenate([vb[rows, :], ones_blk], axis=0)
        kvp = lax.dot_general(vext, pk_pos[rows, :], NT, preferred_element_type=F32)
        kvn = lax.dot_general(vext, pk_neg[rows, :], NT, preferred_element_type=F32)
        kvp = jnp.where(bmask, kvp, 0.0).astype(BF16)
        kvn = jnp.where(bmask, kvn, 0.0).astype(BF16)
        nd = (jnp.dot(kvp, pq_pos[rows, :], preferred_element_type=F32)
              + jnp.dot(kvn, pq_neg[rows, :], preferred_element_type=F32))
        rden = (1.0 - g_row[0:1, :]) / (nd[80:88, :] + 1e-6)
        for p in range(2):
            rE = rden[2 * p: 2 * p + 1, :]; rO = rden[2 * p + 1: 2 * p + 2, :]
            b0 = 40 * p
            o0 = D + 80 * G + b0
            ot[pl.ds(o0, 16), :] = nd[b0: b0 + 16, :] * rE
            ot[pl.ds(o0 + 16, 8), :] = nd[b0 + 16: b0 + 24, :] * jnp.where(lo2, rE, rO)
            ot[pl.ds(o0 + 24, 16), :] = nd[b0 + 24: b0 + 40, :] * rO

    row16 = lax.broadcasted_iota(jnp.int32, (16, TQ), 0)
    lo3 = lax.broadcasted_iota(jnp.int32, (8, TQ), 0) < 4

    def grp(u):
        return ((u & 31) * 43) >> 8

    def prep_qm(u, qm_ref, shift, piece=None):
        t = u >> 5; h = u & 31
        g = grp(u); off = (h - 6 * g) * 20
        cols = pl.ds(pl.multiple_of(t * TQ, TQ), TQ)
        for i in (range(8) if piece is None else (piece,)):
            q = qt[g, 16 * i: 16 * i + 16, cols]
            row = row16 + 16 * i
            qm = jnp.where((row >= off) & (row < off + 20), q, jnp.zeros_like(q))
            if shift and i == BROW // 16:
                b = nb[h >> 1, :, cols]
                qm = jnp.where(row == BROW, jnp.concatenate([b, b], axis=0).astype(BF16), qm)
            qm_ref[16 * i: 16 * i + 16, :] = qm

    def qk_chunk(c, g, qm_ref):
        return jnp.dot(ks[g, c * C:(c + 1) * C, :], qm_ref[...], preferred_element_type=F32)

    def pv_chunk(c, h, p, acc):
        r = jnp.dot(vs[h, :, c * C:(c + 1) * C], rev8(p), preferred_element_type=F32)
        return r if acc is None else acc + r

    def fin(u, acc, odd):
        t = u >> 5; h = u & 31
        cols = pl.ds(pl.multiple_of(t * TQ, TQ), TQ)
        g = g_row[0:1, cols]
        base = pl.multiple_of((h >> 1) * 40, 8)
        if not odd:
            r = g / acc[20:21, :]
            ot[pl.ds(base, 16), cols] = acc[0:16, :] * r
            a_even[...] = acc[16:24, :] * r
        else:
            r = g / acc[0:1, :]
            ot[pl.ds(base + 16, 8), cols] = jnp.where(lo3, a_even[...], acc[0:8, :] * r)
            ot[pl.ds(base + 24, 16), cols] = acc[8:24, :] * r

    safe = jnp.max(bmx[...]) <= BOUND_MAX

    @pl.when(safe)
    def _fast():
        qms = (qm0, qm1, qm2, qm3)
        prep_qm(0, qm0, True)
        prep_qm(1, qm1, True)
        s0[...] = qk_chunk(0, 0, qm0)

        def body(j, carry):
            s = s0[...]
            for r in range(UPB):
                u = UPB * j + r
                odd = r % 2 == 1
                qm_cur, qm_nxt, qm_prep = qms[r % 4], qms[(r + 1) % 4], qms[(r + 2) % 4]
                u1 = jnp.minimum(u + 1, NU - 1)
                u2 = jnp.minimum(u + 2, NU - 1)
                g = grp(u); g1 = grp(u1)
                acc = None
                for c in range(NCH):
                    if c + 1 < NCH:
                        s_next = qk_chunk(c + 1, g, qm_cur)
                    else:
                        s_next = qk_chunk(0, g1, qm_nxt)
                    acc = pv_chunk(c, u & 31, jnp.exp2(s), acc)
                    s = s_next
                    if 4 <= c < 12:
                        prep_qm(u2, qm_prep, True, c - 4)
                fin(u, acc, odd)
            s0[...] = s
            return carry
        lax.fori_loop(0, NU // UPB, body, 0)

    @pl.when(jnp.logical_not(safe))
    def _slow():
        def unit(u, odd):
            g = grp(u); h = u & 31
            prep_qm(u, qm0, False)

            def p1(c, m8):
                r0 = pl.multiple_of(c * C, C)
                s = jnp.dot(ks[g, pl.ds(r0, C), :], qm0[...], preferred_element_type=F32)
                sA[pl.ds(r0, C), :] = s
                return jnp.maximum(m8, jnp.max(s.reshape(C // 8, 8, TQ), axis=0))
            m8 = lax.fori_loop(0, NCH, p1, jnp.full((8, TQ), -jnp.inf, F32))
            m = jnp.max(m8, axis=0, keepdims=True)

            def p2(c, acc):
                r0 = pl.multiple_of(c * C, C)
                p = jnp.exp2(sA[pl.ds(r0, C), :] - m)
                return acc + jnp.dot(vs[h, :, pl.ds(r0, C)], rev8(p), preferred_element_type=F32)
            acc = lax.fori_loop(0, NCH, p2, jnp.zeros((VR, TQ), F32))
            fin(u, acc, odd)

        def body(j, carry):
            unit(2 * j, False)
            unit(2 * j + 1, True)
            return carry
        lax.fori_loop(0, NU // 2, body, 0)

    def outp(t, carry):
        cols = pl.ds(pl.multiple_of(t * TQ, TQ), TQ)
        o = ot[:, cols].astype(BF16)
        y = lax.dot_general(o, wo_v[...], TN, preferred_element_type=F32)
        out_v[cols, :] = y.astype(BF16)
        pltpu.make_async_copy(out_v.at[cols, :], out_hbm.at[cols, :], osems.at[t]).start()
        return carry
    lax.fori_loop(0, NQ, outp, 0)
    for t in range(NQ):
        rows = pl.ds(t * TQ, TQ)
        pltpu.make_async_copy(out_v.at[rows, :], out_hbm.at[rows, :], osems.at[t]).wait()


@jax.jit
def pallas_gated_mix__mha_block__linear_kernel_hedgehog__prompt_kernel(
        A_x, A_wqkv, A_wo, B_x, B_wqkv, B_w_phi, B_wo, gate_w):
    x = A_x.reshape(S, D)
    wphi = jnp.transpose(B_w_phi, (1, 2, 0))
    any_spec = pl.BlockSpec(memory_space=pl.ANY)
    out = pl.pallas_call(
        _kernel,
        out_shape=jax.ShapeDtypeStruct((S, D), BF16),
        in_specs=[any_spec] * 7,
        out_specs=any_spec,
        scratch_shapes=[
            pltpu.VMEM((DH, DH, H), BF16), pltpu.VMEM((D,), BF16),
            pltpu.VMEM((S, D), BF16), pltpu.VMEM((D, D), BF16), pltpu.VMEM((D, D), BF16), pltpu.VMEM((D, D), BF16),
            pltpu.VMEM((D, 3 * D), BF16), pltpu.VMEM((2 * D, D), BF16),
            pltpu.VMEM((D, D), BF16), pltpu.VMEM((LTR, D), BF16),
            pltpu.VMEM((24, D), F32), pltpu.VMEM((D, D), BF16),
            pltpu.VMEM((6, 128, S), BF16), pltpu.VMEM((6, S, 128), BF16), pltpu.VMEM((H, VR, S), F32),
            pltpu.VMEM((D, S), BF16), pltpu.VMEM((D, S), BF16), pltpu.VMEM((D, S), BF16), pltpu.VMEM((D, S), BF16),
            pltpu.VMEM((D, S), BF16), pltpu.VMEM((8, S), F32),
            pltpu.VMEM((16, 8, TP), F32), pltpu.VMEM((16, 8, S), F32), pltpu.VMEM((16, 8, TP), F32),
            pltpu.VMEM((S, TQ), F32), pltpu.VMEM((8, TQ), F32),
            pltpu.VMEM((128, TQ), BF16), pltpu.VMEM((128, TQ), BF16), pltpu.VMEM((128, TQ), BF16),
            pltpu.VMEM((128, TQ), BF16), pltpu.VMEM((C, TQ), F32),
            pltpu.VMEM((2 * D, S), F32), pltpu.VMEM((S, D), BF16),
            pltpu.SemaphoreType.DMA((12,)), pltpu.SemaphoreType.DMA((NQ,)),
        ],
        compiler_params=pltpu.CompilerParams(vmem_limit_bytes=110 * 1024 * 1024),
    )(x, A_wqkv, A_wo, B_wqkv, wphi, B_wo, gate_w)
    return out.reshape(1, S, D)
```

```python
import math

import jax
import jax.numpy as jnp
from jax import lax
from jax.experimental import pallas as pl
from jax.experimental.pallas import tpu as pltpu

S = 2048; D = 640; H = 32; DH = 20
TQ = 512; NQ = S // TQ
C = 128; NCH = S // C
UPB = 8
NU = NQ * H
VR = 24
F32 = jnp.float32; BF16 = jnp.bfloat16
LOG2E = math.log2(math.e)
QSCALE = (DH ** -0.5) * LOG2E
BOUND_MAX = 30.0
NT = (((1,), (1,)), ((), ()))
TN = (((0,), (0,)), ((), ()))
TP = 512
LTR = 5 * D + 16
BAND = [((80 * G) // 128, (80 * G + 79) // 128 + 1) for G in range(8)]
R_PQ, R_PK, R_Q, R_VA, R_G, R_VB = 0, D, 2 * D, 3 * D, 4 * D, 4 * D + 16
BROW = 120


def _kernel(x_hbm, wa_hbm, woa_hbm, wb_hbm, wphi_hbm, wob_hbm, gate_hbm, out_hbm,
            wphi_ref, gate_ref, x_v, wak_v, waq_v, wav_v, wb_v, wo_v,
            wkt, lt, mscr, tbd, qt, ks, vs, pq_pos, pq_neg, pk_pos, pk_neg, vb, g_row,
            kn, nb, bmx,
            sA, a_even, qm0, qm1, qm2, qm3, s0, ot, out_v, sems, osems):
    cp_wk = pltpu.make_async_copy(wa_hbm.at[:, D:2 * D], wak_v, sems.at[0])
    cp_x = [pltpu.make_async_copy(x_hbm.at[pl.ds(i * TP, TP), :], x_v.at[pl.ds(i * TP, TP), :], sems.at[1 + i])
            for i in range(4)]
    cp_wq = pltpu.make_async_copy(wa_hbm.at[:, 0:D], waq_v, sems.at[9])
    cp_wav = pltpu.make_async_copy(wa_hbm.at[:, 2 * D:3 * D], wav_v, sems.at[5])
    cp_wb = pltpu.make_async_copy(wb_hbm, wb_v, sems.at[6])
    cp_woa = pltpu.make_async_copy(woa_hbm, wo_v.at[0:D, :], sems.at[7])
    cp_wob = pltpu.make_async_copy(wob_hbm, wo_v.at[D:2 * D, :], sems.at[8])
    cp_phi = pltpu.make_async_copy(wphi_hbm, wphi_ref, sems.at[10])
    cp_gate = pltpu.make_async_copy(gate_hbm, gate_ref, sems.at[11])
    cp_phi.start()
    cp_wk.start()
    cp_x[0].start()
    cp_gate.start()
    cp_phi.wait()

    for d in range(DH):
        mscr[0:DH, 32 * d: 32 * d + 32] = wphi_ref[d].astype(F32)
    m1 = mscr[0:DH, :].astype(BF16)
    pi = lax.broadcasted_iota(jnp.int32, (D, D), 0)
    pj = lax.broadcasted_iota(jnp.int32, (D, D), 1)
    perm = jnp.where(pj == 20 * (pi & 31) + (pi >> 5), 1.0, 0.0).astype(BF16)
    m2 = jnp.dot(m1, perm, preferred_element_type=F32).astype(BF16)
    ei = lax.broadcasted_iota(jnp.int32, (D, DH), 0)
    ej = lax.broadcasted_iota(jnp.int32, (D, DH), 1)
    et = jnp.where(((ei - 80 * ((ei * 3277) >> 18)) >> 2) == ej, 1.0, 0.0).astype(BF16)
    tiled = jnp.dot(et, m2, preferred_element_type=F32)
    same = (4 * ((pi * 3277) >> 18) + (pi & 3)) == ((pj * 3277) >> 16)
    tbd[...] = jnp.where(same, tiled, 0.0).astype(BF16)

    for cp in cp_x[1:]:
        cp.start()
    cp_wq.start(); cp_wav.start(); cp_wb.start(); cp_woa.start(); cp_wob.start()

    sub = lax.broadcasted_iota(jnp.int32, (16, 8, TP), 1)
    lo = sub < 4

    def tr(w):
        return w.astype(F32).T.astype(BF16)

    def pairnorm(y):
        y3 = y.reshape(16, 40, TP)
        return jnp.sum(y3 * y3, axis=1, keepdims=True)

    def rev8(a):
        n = a.shape[0]
        return jnp.concatenate([a[128 * b + 8 * (15 - j): 128 * b + 8 * (15 - j) + 8, :]
                                for b in range(n // 128) for j in range(16)], axis=0)

    def k_proj(tt):
        rows = pl.ds(tt * TP if isinstance(tt, int) else pl.multiple_of(tt * TP, TP), TP)
        kt = lax.dot_general(wkt[...], x_v[rows, :], NT, preferred_element_type=F32)
        for g in range(6):
            w = min(120, D - 120 * g)
            parts = [kt[120 * g: 120 * g + w, :]]
            if w < BROW:
                parts.append(jnp.zeros((BROW - w, TP), F32))
            parts.append(jnp.where(lax.broadcasted_iota(jnp.int32, (8, TP), 0) == 0, 1.0, 0.0))
            ks[g, rows, :] = rev8(jnp.concatenate(parts, axis=0).T).astype(BF16)
        n = jnp.broadcast_to(pairnorm(kt), (16, 8, TP))
        kn[...] = n if isinstance(tt, int) and tt == 0 else jnp.maximum(kn[...], n)

    def fold(off, row0):
        for j, (k0, k1) in enumerate(BAND):
            r = lax.dot_general(tbd[80 * j: 80 * j + 80, 128 * k0: 128 * k1],
                                wb_v[:, off + 128 * k0: off + 128 * k1], NT, preferred_element_type=F32)
            lt[row0 + 80 * j: row0 + 80 * j + 80, :] = (r * LOG2E).astype(BF16)

    cp_wk.wait()
    wkt[...] = tr(wak_v[...])
    cp_x[0].wait()
    k_proj(0)
    cp_x[1].wait(); cp_x[2].wait()
    lax.fori_loop(1, 3, lambda tt, c: (k_proj(tt), c)[1], 0)
    cp_x[3].wait(); cp_wq.wait(); cp_wav.wait()
    lt[R_Q:R_Q + D, :] = tr(waq_v[...])
    k_proj(3)
    lt[R_VA:R_VA + D, :] = tr(wav_v[...])
    cp_wb.wait(); cp_gate.wait()
    fold(0, R_PQ)
    lt[R_VB:R_VB + D, :] = tr(wb_v[:, 2 * D:3 * D])
    fold(D, R_PK)
    lt[R_G:R_G + 16, :] = jnp.broadcast_to(gate_ref[...].astype(F32).reshape(1, D), (16, D)).astype(BF16)
    for g in range(6):
        w = min(120, D - 120 * g)
        qt[g, w:128, :] = jnp.zeros((128 - w, S), BF16)
    kn[...] = jnp.broadcast_to(jnp.max(kn[...], axis=2, keepdims=True), (16, 8, TP))
    bmx[...] = jnp.zeros_like(bmx)

    def feat(y, pos_ref, neg_ref, cols):
        y4 = y.reshape(8, 10, 8, TP)
        mx = jnp.max(y4, axis=1); mx = jnp.maximum(mx, pltpu.roll(mx, 4, 1))[:, None]
        mn = jnp.min(y4, axis=1); mn = jnp.minimum(mn, pltpu.roll(mn, 4, 1))[:, None]
        for e, ref in ((jnp.exp2(y4 - mx), pos_ref), (jnp.exp2(mn - y4), neg_ref)):
            s = jnp.sum(e, axis=1); s = s + pltpu.roll(s, 4, 1)
            ref[:, cols] = (e * (1.0 / s)[:, None]).reshape(D, TP).astype(BF16)

    def proj(tt, carry):
        cols = pl.ds(pl.multiple_of(tt * TP, TP), TP)
        yt = lax.dot_general(lt[...], x_v[cols, :], NT, preferred_element_type=F32)
        v3 = yt[R_VA:R_VA + D, :].reshape(16, 40, TP)
        a = [v3[:, 8 * i: 8 * i + 8, :] for i in range(5)]
        e2 = jnp.where(lo, a[2], jnp.where(sub == 4, 1.0, 0.0))
        o0 = jnp.where(lo, jnp.where(sub == 0, 1.0, 0.0), a[2])
        ve = jnp.concatenate([a[0], a[1], e2, o0, a[3], a[4]], axis=1)
        vs[:, :, cols] = ve.reshape(H, VR, TP)
        feat(yt[R_PQ:R_PQ + D, :], pq_pos, pq_neg, cols)
        feat(yt[R_PK:R_PK + D, :], pk_pos, pk_neg, cols)
        vb[:, cols] = yt[R_VB:R_VB + D, :].astype(BF16)
        q = yt[R_Q:R_Q + D, :] * QSCALE
        for g in range(6):
            w = min(120, D - 120 * g)
            qt[g, 0:w, cols] = q[120 * g: 120 * g + w, :].astype(BF16)
        bnd = jnp.sqrt(pairnorm(q) * kn[...])
        nb[:, :, cols] = -bnd
        bmx[...] = jnp.maximum(bmx[...], bnd)
        z = yt[R_G:R_G + 8, :]
        g_row[:, cols] = 1.0 / (1.0 + jnp.exp(-z))
        return carry
    lax.fori_loop(0, S // TP, proj, 0)

    cp_woa.wait()
    cp_wob.wait()
    rr = lax.broadcasted_iota(jnp.int32, (96, 80), 0)
    cc = lax.broadcasted_iota(jnp.int32, (96, 80), 1) & 3
    hrow = jnp.where(rr < 80, (rr * 3277) >> 16, rr - 80)
    bmask = hrow == cc
    lo2 = lax.broadcasted_iota(jnp.int32, (8, S), 0) < 4
    for G in range(8):
        rows = pl.ds(80 * G, 80)
        ones_blk = jnp.where(lax.broadcasted_iota(jnp.int32, (16, S), 0) < 4, 1.0, 0.0).astype(BF16)
        vext = jnp.concatenate([vb[rows, :], ones_blk], axis=0)
        kvp = lax.dot_general(vext, pk_pos[rows, :], NT, preferred_element_type=F32)
        kvn = lax.dot_general(vext, pk_neg[rows, :], NT, preferred_element_type=F32)
        kvp = jnp.where(bmask, kvp, 0.0).astype(BF16)
        kvn = jnp.where(bmask, kvn, 0.0).astype(BF16)
        nd = (jnp.dot(kvp, pq_pos[rows, :], preferred_element_type=F32)
              + jnp.dot(kvn, pq_neg[rows, :], preferred_element_type=F32))
        rden = (1.0 - g_row[0:1, :]) / (nd[80:88, :] + 1e-6)
        for p in range(2):
            rE = rden[2 * p: 2 * p + 1, :]; rO = rden[2 * p + 1: 2 * p + 2, :]
            b0 = 40 * p
            o0 = D + 80 * G + b0
            ot[pl.ds(o0, 16), :] = nd[b0: b0 + 16, :] * rE
            ot[pl.ds(o0 + 16, 8), :] = nd[b0 + 16: b0 + 24, :] * jnp.where(lo2, rE, rO)
            ot[pl.ds(o0 + 24, 16), :] = nd[b0 + 24: b0 + 40, :] * rO

    row16 = lax.broadcasted_iota(jnp.int32, (16, TQ), 0)
    lo3 = lax.broadcasted_iota(jnp.int32, (8, TQ), 0) < 4

    def grp(u):
        return ((u & 31) * 43) >> 8

    def prep_qm(u, qm_ref, shift, piece=None):
        t = u >> 5; h = u & 31
        g = grp(u); off = (h - 6 * g) * 20
        cols = pl.ds(pl.multiple_of(t * TQ, TQ), TQ)
        for i in (range(8) if piece is None else (piece,)):
            q = qt[g, 16 * i: 16 * i + 16, cols]
            row = row16 + 16 * i
            qm = jnp.where((row >= off) & (row < off + 20), q, jnp.zeros_like(q))
            if shift and i == BROW // 16:
                b = nb[h >> 1, :, cols]
                qm = jnp.where(row == BROW, jnp.concatenate([b, b], axis=0).astype(BF16), qm)
            qm_ref[16 * i: 16 * i + 16, :] = qm

    def qk_chunk(c, g, qm_ref):
        return jnp.dot(ks[g, c * C:(c + 1) * C, :], qm_ref[...], preferred_element_type=F32)

    def pv_chunk(c, h, p, acc):
        r = jnp.dot(vs[h, :, c * C:(c + 1) * C], rev8(p), preferred_element_type=F32)
        return r if acc is None else acc + r

    def fin(u, acc, odd):
        t = u >> 5; h = u & 31
        cols = pl.ds(pl.multiple_of(t * TQ, TQ), TQ)
        g = g_row[0:1, cols]
        base = pl.multiple_of((h >> 1) * 40, 8)
        if not odd:
            r = g / acc[20:21, :]
            ot[pl.ds(base, 16), cols] = acc[0:16, :] * r
            a_even[...] = acc[16:24, :] * r
        else:
            r = g / acc[0:1, :]
            ot[pl.ds(base + 16, 8), cols] = jnp.where(lo3, a_even[...], acc[0:8, :] * r)
            ot[pl.ds(base + 24, 16), cols] = acc[8:24, :] * r

    safe = jnp.max(bmx[...]) <= BOUND_MAX

    @pl.when(safe)
    def _fast():
        qms = (qm0, qm1, qm2, qm3)
        prep_qm(0, qm0, True)
        prep_qm(1, qm1, True)
        s0[...] = qk_chunk(0, 0, qm0)

        def body(j, carry):
            s = s0[...]
            for r in range(UPB):
                u = UPB * j + r
                odd = r % 2 == 1
                qm_cur, qm_nxt, qm_prep = qms[r % 4], qms[(r + 1) % 4], qms[(r + 2) % 4]
                u1 = jnp.minimum(u + 1, NU - 1)
                u2 = jnp.minimum(u + 2, NU - 1)
                g = grp(u); g1 = grp(u1)
                acc = None
                for c in range(NCH):
                    if c + 1 < NCH:
                        s_next = qk_chunk(c + 1, g, qm_cur)
                    else:
                        s_next = qk_chunk(0, g1, qm_nxt)
                    acc = pv_chunk(c, u & 31, jnp.exp2(s), acc)
                    s = s_next
                    if 4 <= c < 12:
                        prep_qm(u2, qm_prep, True, c - 4)
                fin(u, acc, odd)
            s0[...] = s
            return carry
        lax.fori_loop(0, NU // UPB, body, 0)

    @pl.when(jnp.logical_not(safe))
    def _slow():
        def unit(u, carry):
            g = grp(u); h = u & 31
            prep_qm(u, qm0, False)

            def p1(c, m8):
                r0 = pl.multiple_of(c * C, C)
                s = jnp.dot(ks[g, pl.ds(r0, C), :], qm0[...], preferred_element_type=F32)
                sA[pl.ds(r0, C), :] = s
                return jnp.maximum(m8, jnp.max(s.reshape(C // 8, 8, TQ), axis=0))
            m8 = lax.fori_loop(0, NCH, p1, jnp.full((8, TQ), -jnp.inf, F32))
            m = jnp.max(m8, axis=0, keepdims=True)

            def p2(c, acc):
                r0 = pl.multiple_of(c * C, C)
                p = jnp.exp2(sA[pl.ds(r0, C), :] - m)
                return acc + jnp.dot(vs[h, :, pl.ds(r0, C)], rev8(p), preferred_element_type=F32)
            acc = lax.fori_loop(0, NCH, p2, jnp.zeros((VR, TQ), F32))
            pl.when((u & 1) == 0)(lambda: fin(u, acc, False))
            pl.when((u & 1) == 1)(lambda: fin(u, acc, True))
            return carry
        lax.fori_loop(0, NU, unit, 0)

    def outp(t, carry):
        cols = pl.ds(pl.multiple_of(t * TQ, TQ), TQ)
        o = ot[:, cols].astype(BF16)
        y = lax.dot_general(o, wo_v[...], TN, preferred_element_type=F32)
        out_v[cols, :] = y.astype(BF16)
        pltpu.make_async_copy(out_v.at[cols, :], out_hbm.at[cols, :], osems.at[t]).start()
        return carry
    lax.fori_loop(0, NQ, outp, 0)
    for t in range(NQ):
        rows = pl.ds(t * TQ, TQ)
        pltpu.make_async_copy(out_v.at[rows, :], out_hbm.at[rows, :], osems.at[t]).wait()


@jax.jit
def pallas_gated_mix__mha_block__linear_kernel_hedgehog__prompt_kernel(
        A_x, A_wqkv, A_wo, B_x, B_wqkv, B_w_phi, B_wo, gate_w):
    x = A_x.reshape(S, D)
    wphi = jnp.transpose(B_w_phi, (1, 2, 0))
    any_spec = pl.BlockSpec(memory_space=pl.ANY)
    out = pl.pallas_call(
        _kernel,
        out_shape=jax.ShapeDtypeStruct((S, D), BF16),
        in_specs=[any_spec] * 7,
        out_specs=any_spec,
        scratch_shapes=[
            pltpu.VMEM((DH, DH, H), BF16), pltpu.VMEM((D,), BF16),
            pltpu.VMEM((S, D), BF16), pltpu.VMEM((D, D), BF16), pltpu.VMEM((D, D), BF16), pltpu.VMEM((D, D), BF16),
            pltpu.VMEM((D, 3 * D), BF16), pltpu.VMEM((2 * D, D), BF16),
            pltpu.VMEM((D, D), BF16), pltpu.VMEM((LTR, D), BF16),
            pltpu.VMEM((24, D), F32), pltpu.VMEM((D, D), BF16),
            pltpu.VMEM((6, 128, S), BF16), pltpu.VMEM((6, S, 128), BF16), pltpu.VMEM((H, VR, S), F32),
            pltpu.VMEM((D, S), BF16), pltpu.VMEM((D, S), BF16), pltpu.VMEM((D, S), BF16), pltpu.VMEM((D, S), BF16),
            pltpu.VMEM((D, S), BF16), pltpu.VMEM((8, S), F32),
            pltpu.VMEM((16, 8, TP), F32), pltpu.VMEM((16, 8, S), F32), pltpu.VMEM((16, 8, TP), F32),
            pltpu.VMEM((S, TQ), F32), pltpu.VMEM((8, TQ), F32),
            pltpu.VMEM((128, TQ), BF16), pltpu.VMEM((128, TQ), BF16), pltpu.VMEM((128, TQ), BF16),
            pltpu.VMEM((128, TQ), BF16), pltpu.VMEM((C, TQ), F32),
            pltpu.VMEM((2 * D, S), F32), pltpu.VMEM((S, D), BF16),
            pltpu.SemaphoreType.DMA((12,)), pltpu.SemaphoreType.DMA((NQ,)),
        ],
        compiler_params=pltpu.CompilerParams(vmem_limit_bytes=110 * 1024 * 1024),
    )(x, A_wqkv, A_wo, B_wqkv, wphi, B_wo, gate_w)
    return out.reshape(1, S, D)
```

```python
import math

import jax
import jax.numpy as jnp
from jax import lax
from jax.experimental import pallas as pl
from jax.experimental.pallas import tpu as pltpu

S = 2048; D = 640; H = 32; DH = 20
TQ = 512; NQ = S // TQ
C = 128; NCH = S // C
UPB = 8
NU = NQ * H
VR = 24
F32 = jnp.float32; BF16 = jnp.bfloat16; U32 = jnp.uint32
LOG2E = math.log2(math.e)
QSCALE = (DH ** -0.5) * LOG2E
BOUND_MAX = 30.0
NT = (((1,), (1,)), ((), ()))
TN = (((0,), (0,)), ((), ()))
TP = 512
LTR = 5 * D + 16
BAND = [((80 * G) // 128, (80 * G + 79) // 128 + 1) for G in range(8)]
R_PQ, R_PK, R_Q, R_VA, R_G, R_VB = 0, D, 2 * D, 3 * D, 4 * D, 4 * D + 16


def _kernel(x_hbm, wa_hbm, woa_hbm, wb_hbm, wphi_hbm, wob_hbm, gate_hbm, out_hbm,
            wphi_ref, gate_ref, x_v, wak_v, waq_v, wav_v, wb_v, wo_v,
            wkt, lt, mscr, tbd, qt, ks, kh, vs, pq_pos, pq_neg, pk_pos, pk_neg, vb, g_row,
            kn, bmx,
            sA, a_even, s0, ot, out_v, sems, osems):
    cp_wk = pltpu.make_async_copy(wa_hbm.at[:, D:2 * D], wak_v, sems.at[0])
    cp_x = [pltpu.make_async_copy(x_hbm.at[pl.ds(i * TP, TP), :], x_v.at[pl.ds(i * TP, TP), :], sems.at[1 + i])
            for i in range(4)]
    cp_wq = pltpu.make_async_copy(wa_hbm.at[:, 0:D], waq_v, sems.at[9])
    cp_wav = pltpu.make_async_copy(wa_hbm.at[:, 2 * D:3 * D], wav_v, sems.at[5])
    cp_wb = pltpu.make_async_copy(wb_hbm, wb_v, sems.at[6])
    cp_woa = pltpu.make_async_copy(woa_hbm, wo_v.at[0:D, :], sems.at[7])
    cp_wob = pltpu.make_async_copy(wob_hbm, wo_v.at[D:2 * D, :], sems.at[8])
    cp_phi = pltpu.make_async_copy(wphi_hbm, wphi_ref, sems.at[10])
    cp_gate = pltpu.make_async_copy(gate_hbm, gate_ref, sems.at[11])
    cp_phi.start()
    cp_wk.start()
    cp_x[0].start()
    cp_gate.start()
    cp_phi.wait()

    for d in range(DH):
        mscr[0:DH, 32 * d: 32 * d + 32] = wphi_ref[d].astype(F32)
    m1 = mscr[0:DH, :].astype(BF16)
    pi = lax.broadcasted_iota(jnp.int32, (D, D), 0)
    pj = lax.broadcasted_iota(jnp.int32, (D, D), 1)
    perm = jnp.where(pj == 20 * (pi & 31) + (pi >> 5), 1.0, 0.0).astype(BF16)
    m2 = jnp.dot(m1, perm, preferred_element_type=F32).astype(BF16)
    ei = lax.broadcasted_iota(jnp.int32, (D, DH), 0)
    ej = lax.broadcasted_iota(jnp.int32, (D, DH), 1)
    et = jnp.where(((ei - 80 * ((ei * 3277) >> 18)) >> 2) == ej, 1.0, 0.0).astype(BF16)
    tiled = jnp.dot(et, m2, preferred_element_type=F32)
    same = (4 * ((pi * 3277) >> 18) + (pi & 3)) == ((pj * 3277) >> 16)
    tbd[...] = jnp.where(same, tiled, 0.0).astype(BF16)

    for cp in cp_x[1:]:
        cp.start()
    cp_wq.start(); cp_wav.start(); cp_wb.start(); cp_woa.start(); cp_wob.start()

    sub = lax.broadcasted_iota(jnp.int32, (16, 8, TP), 1)
    lo = sub < 4

    def pk32(v):
        return pltpu.bitcast(v, U32)

    def up32(v):
        return pltpu.bitcast(v, BF16)

    def tr(w):
        return pk32(w.astype(F32).T.astype(BF16))

    def pairnorm(y):
        y3 = y.reshape(16, 40, TP)
        return jnp.sum(y3 * y3, axis=1, keepdims=True)

    def rev8(a):
        n = a.shape[0]
        return jnp.concatenate([a[128 * b + 8 * (15 - j): 128 * b + 8 * (15 - j) + 8, :]
                                for b in range(n // 128) for j in range(16)], axis=0)

    def ext32(y, fill):
        v3 = y.reshape(16, 40, TP)
        a = [v3[:, 8 * i: 8 * i + 8, :] for i in range(5)]
        z = jnp.zeros((16, 8, TP), F32)
        e2 = jnp.where(lo, a[2], jnp.where(sub == 4, fill, 0.0))
        o0 = jnp.where(lo, jnp.where(sub == 0, fill, 0.0), a[2])
        return jnp.concatenate([a[0], a[1], e2, z, o0, a[3], a[4], z], axis=1)

    def k_proj(tt):
        rows = pl.ds(tt * TP if isinstance(tt, int) else pl.multiple_of(tt * TP, TP), TP)
        hrows = pl.ds(tt * (TP // 2) if isinstance(tt, int) else pl.multiple_of(tt * (TP // 2), TP // 2), TP // 2)
        kt = lax.dot_general(up32(wkt[...]), x_v[rows, :], NT, preferred_element_type=F32)
        ke = ext32(kt, 1.0).reshape(8, 128, TP)
        for G in range(8):
            ks[G, hrows, :] = pk32(rev8(ke[G].T).astype(BF16))
        n = jnp.broadcast_to(pairnorm(kt), (16, 8, TP))
        kn[...] = n if isinstance(tt, int) and tt == 0 else jnp.maximum(kn[...], n)

    def fold(off, row0):
        for j, (k0, k1) in enumerate(BAND):
            r = lax.dot_general(tbd[80 * j: 80 * j + 80, 128 * k0: 128 * k1],
                                wb_v[:, off + 128 * k0: off + 128 * k1], NT, preferred_element_type=F32)
            lt[(row0 + 80 * j) // 2: (row0 + 80 * j + 80) // 2, :] = pk32((r * LOG2E).astype(BF16))

    cp_wk.wait()
    wkt[...] = tr(wak_v[...])
    cp_x[0].wait()
    k_proj(0)
    cp_x[1].wait(); cp_x[2].wait()
    lax.fori_loop(1, 3, lambda tt, c: (k_proj(tt), c)[1], 0)
    cp_x[3].wait(); cp_wq.wait(); cp_wav.wait()
    lt[R_Q // 2:(R_Q + D) // 2, :] = tr(waq_v[...])
    k_proj(3)
    lt[R_VA // 2:(R_VA + D) // 2, :] = tr(wav_v[...])
    cp_wb.wait(); cp_gate.wait()
    fold(0, R_PQ)
    lt[R_VB // 2:(R_VB + D) // 2, :] = tr(wb_v[:, 2 * D:3 * D])
    fold(D, R_PK)
    lt[R_G // 2:(R_G + 16) // 2, :] = pk32(jnp.broadcast_to(gate_ref[...].astype(F32).reshape(1, D), (16, D)).astype(BF16))
    kn[...] = jnp.broadcast_to(jnp.max(kn[...], axis=2, keepdims=True), (16, 8, TP))
    bmx[...] = jnp.zeros_like(bmx)

    def feat(y, pos_ref, neg_ref, cols):
        y4 = y.reshape(8, 10, 8, TP)
        mx = jnp.max(y4, axis=1); mx = jnp.maximum(mx, pltpu.roll(mx, 4, 1))[:, None]
        mn = jnp.min(y4, axis=1); mn = jnp.minimum(mn, pltpu.roll(mn, 4, 1))[:, None]
        for e, ref in ((jnp.exp2(y4 - mx), pos_ref), (jnp.exp2(mn - y4), neg_ref)):
            s = jnp.sum(e, axis=1); s = s + pltpu.roll(s, 4, 1)
            ref[:, cols] = (e * (1.0 / s)[:, None]).reshape(D, TP).astype(BF16)

    def proj(tt, carry):
        cols = pl.ds(pl.multiple_of(tt * TP, TP), TP)
        yt = lax.dot_general(up32(lt[...]), x_v[cols, :], NT, preferred_element_type=F32)
        v3 = yt[R_VA:R_VA + D, :].reshape(16, 40, TP)
        a = [v3[:, 8 * i: 8 * i + 8, :] for i in range(5)]
        e2 = jnp.where(lo, a[2], jnp.where(sub == 4, 1.0, 0.0))
        o0 = jnp.where(lo, jnp.where(sub == 0, 1.0, 0.0), a[2])
        ve = jnp.concatenate([a[0], a[1], e2, o0, a[3], a[4]], axis=1)
        vs[:, :, cols] = ve.reshape(H, VR, TP)
        feat(yt[R_PQ:R_PQ + D, :], pq_pos, pq_neg, cols)
        feat(yt[R_PK:R_PK + D, :], pk_pos, pk_neg, cols)
        vb[:, cols] = yt[R_VB:R_VB + D, :].astype(BF16)
        q = yt[R_Q:R_Q + D, :] * QSCALE
        bnd = jnp.sqrt(pairnorm(q) * kn[...])
        qe = ext32(q, -bnd).reshape(H * 32, TP).astype(BF16)
        qt[:, :, cols] = pk32(qe).reshape(H, 16, TP)
        bmx[...] = jnp.maximum(bmx[...], bnd)
        hrows = pl.ds(pl.multiple_of(tt * (TP // 2), TP // 2), TP // 2)
        for G in range(8):
            t4 = ks[G, hrows, :]
            for jj in range(4):
                kh[4 * G + jj, hrows, :] = t4 if jj == 0 else pltpu.roll(t4, 128 - 32 * jj, 1)
        z = yt[R_G:R_G + 8, :]
        g_row[:, cols] = 1.0 / (1.0 + jnp.exp(-z))
        return carry
    lax.fori_loop(0, S // TP, proj, 0)

    cp_woa.wait()
    cp_wob.wait()
    rr = lax.broadcasted_iota(jnp.int32, (96, 80), 0)
    cc = lax.broadcasted_iota(jnp.int32, (96, 80), 1) & 3
    hrow = jnp.where(rr < 80, (rr * 3277) >> 16, rr - 80)
    bmask = hrow == cc
    lo2 = lax.broadcasted_iota(jnp.int32, (8, S), 0) < 4
    for G in range(8):
        rows = pl.ds(80 * G, 80)
        ones_blk = jnp.where(lax.broadcasted_iota(jnp.int32, (16, S), 0) < 4, 1.0, 0.0).astype(BF16)
        vext = jnp.concatenate([vb[rows, :], ones_blk], axis=0)
        kvp = lax.dot_general(vext, pk_pos[rows, :], NT, preferred_element_type=F32)
        kvn = lax.dot_general(vext, pk_neg[rows, :], NT, preferred_element_type=F32)
        kvp = jnp.where(bmask, kvp, 0.0).astype(BF16)
        kvn = jnp.where(bmask, kvn, 0.0).astype(BF16)
        nd = (jnp.dot(kvp, pq_pos[rows, :], preferred_element_type=F32)
              + jnp.dot(kvn, pq_neg[rows, :], preferred_element_type=F32))
        rden = (1.0 - g_row[0:1, :]) / (nd[80:88, :] + 1e-6)
        for p in range(2):
            rE = rden[2 * p: 2 * p + 1, :]; rO = rden[2 * p + 1: 2 * p + 2, :]
            b0 = 40 * p
            o0 = D + 80 * G + b0
            ot[pl.ds(o0, 16), :] = nd[b0: b0 + 16, :] * rE
            ot[pl.ds(o0 + 16, 8), :] = nd[b0 + 16: b0 + 24, :] * jnp.where(lo2, rE, rO)
            ot[pl.ds(o0 + 24, 16), :] = nd[b0 + 24: b0 + 40, :] * rO

    lo3 = lax.broadcasted_iota(jnp.int32, (8, TQ), 0) < 4

    def qcols(u):
        return pl.ds(pl.multiple_of((u >> 5) * TQ, TQ), TQ)

    def qk_chunk(c, u):
        h = u & 31
        return jnp.dot(up32(kh[h, c * (C // 2):(c + 1) * (C // 2), 0:32]), up32(qt[h, :, qcols(u)]),
                       preferred_element_type=F32)

    def pv_chunk(c, h, p, acc):
        r = jnp.dot(vs[h, :, c * C:(c + 1) * C], rev8(p), preferred_element_type=F32)
        return r if acc is None else acc + r

    def fin(u, acc, odd):
        t = u >> 5; h = u & 31
        cols = pl.ds(pl.multiple_of(t * TQ, TQ), TQ)
        g = g_row[0:1, cols]
        base = pl.multiple_of((h >> 1) * 40, 8)
        if not odd:
            r = g / acc[20:21, :]
            ot[pl.ds(base, 16), cols] = acc[0:16, :] * r
            a_even[...] = acc[16:24, :] * r
        else:
            r = g / acc[0:1, :]
            ot[pl.ds(base + 16, 8), cols] = jnp.where(lo3, a_even[...], acc[0:8, :] * r)
            ot[pl.ds(base + 24, 16), cols] = acc[8:24, :] * r

    safe = jnp.max(bmx[...]) <= BOUND_MAX

    @pl.when(safe)
    def _fast():
        s0[...] = qk_chunk(0, 0)

        def body(j, carry):
            s = s0[...]
            for r in range(UPB):
                u = UPB * j + r
                u1 = jnp.minimum(u + 1, NU - 1)
                acc = None
                for c in range(NCH):
                    s_next = qk_chunk(c + 1, u) if c + 1 < NCH else qk_chunk(0, u1)
                    acc = pv_chunk(c, u & 31, jnp.exp2(s), acc)
                    s = s_next
                fin(u, acc, r % 2 == 1)
            s0[...] = s
            return carry
        lax.fori_loop(0, NU // UPB, body, 0)

    @pl.when(jnp.logical_not(safe))
    def _slow():
        def unit(u, carry):
            h = u & 31
            q = up32(qt[h, :, qcols(u)])
            shift_row = jnp.where((h & 1) == 1, 0, 20)
            q = jnp.where(lax.broadcasted_iota(jnp.int32, (32, TQ), 0) == shift_row, jnp.zeros_like(q), q)

            def p1(c, m8):
                r0 = pl.multiple_of(c * C, C)
                kc = kh[h, pl.ds(pl.multiple_of(c * (C // 2), C // 2), C // 2), 0:32]
                s = jnp.dot(up32(kc), q, preferred_element_type=F32)
                sA[pl.ds(r0, C), :] = s
                return jnp.maximum(m8, jnp.max(s.reshape(C // 8, 8, TQ), axis=0))
            m8 = lax.fori_loop(0, NCH, p1, jnp.full((8, TQ), -jnp.inf, F32))
            m = jnp.max(m8, axis=0, keepdims=True)

            def p2(c, acc):
                r0 = pl.multiple_of(c * C, C)
                p = jnp.exp2(sA[pl.ds(r0, C), :] - m)
                return acc + jnp.dot(vs[h, :, pl.ds(r0, C)], rev8(p), preferred_element_type=F32)
            acc = lax.fori_loop(0, NCH, p2, jnp.zeros((VR, TQ), F32))
            pl.when((u & 1) == 0)(lambda: fin(u, acc, False))
            pl.when((u & 1) == 1)(lambda: fin(u, acc, True))
            return carry
        lax.fori_loop(0, NU, unit, 0)

    def outp(t, carry):
        cols = pl.ds(pl.multiple_of(t * TQ, TQ), TQ)
        o = ot[:, cols].astype(BF16)
        y = lax.dot_general(o, wo_v[...], TN, preferred_element_type=F32)
        out_v[cols, :] = y.astype(BF16)
        pltpu.make_async_copy(out_v.at[cols, :], out_hbm.at[cols, :], osems.at[t]).start()
        return carry
    lax.fori_loop(0, NQ, outp, 0)
    for t in range(NQ):
        rows = pl.ds(t * TQ, TQ)
        pltpu.make_async_copy(out_v.at[rows, :], out_hbm.at[rows, :], osems.at[t]).wait()


@jax.jit
def pallas_gated_mix__mha_block__linear_kernel_hedgehog__prompt_kernel(
        A_x, A_wqkv, A_wo, B_x, B_wqkv, B_w_phi, B_wo, gate_w):
    x = A_x.reshape(S, D)
    wphi = jnp.transpose(B_w_phi, (1, 2, 0))
    any_spec = pl.BlockSpec(memory_space=pl.ANY)
    out = pl.pallas_call(
        _kernel,
        out_shape=jax.ShapeDtypeStruct((S, D), BF16),
        in_specs=[any_spec] * 7,
        out_specs=any_spec,
        scratch_shapes=[
            pltpu.VMEM((DH, DH, H), BF16), pltpu.VMEM((D,), BF16),
            pltpu.VMEM((S, D), BF16), pltpu.VMEM((D, D), BF16), pltpu.VMEM((D, D), BF16), pltpu.VMEM((D, D), BF16),
            pltpu.VMEM((D, 3 * D), BF16), pltpu.VMEM((2 * D, D), BF16),
            pltpu.VMEM((D // 2, D), U32), pltpu.VMEM((LTR // 2, D), U32),
            pltpu.VMEM((24, D), F32), pltpu.VMEM((D, D), BF16),
            pltpu.VMEM((H, 16, S), U32), pltpu.VMEM((8, S // 2, 128), U32), pltpu.VMEM((H, S // 2, 128), U32), pltpu.VMEM((H, VR, S), F32),
            pltpu.VMEM((D, S), BF16), pltpu.VMEM((D, S), BF16), pltpu.VMEM((D, S), BF16), pltpu.VMEM((D, S), BF16),
            pltpu.VMEM((D, S), BF16), pltpu.VMEM((8, S), F32),
            pltpu.VMEM((16, 8, TP), F32), pltpu.VMEM((16, 8, TP), F32),
            pltpu.VMEM((S, TQ), F32), pltpu.VMEM((8, TQ), F32),
            pltpu.VMEM((C, TQ), F32),
            pltpu.VMEM((2 * D, S), F32), pltpu.VMEM((S, D), BF16),
            pltpu.SemaphoreType.DMA((12,)), pltpu.SemaphoreType.DMA((NQ,)),
        ],
        compiler_params=pltpu.CompilerParams(vmem_limit_bytes=110 * 1024 * 1024),
    )(x, A_wqkv, A_wo, B_wqkv, wphi, B_wo, gate_w)
    return out.reshape(1, S, D)
```

```python
import math

import jax
import jax.numpy as jnp
from jax import lax
from jax.experimental import pallas as pl
from jax.experimental.pallas import tpu as pltpu

S = 2048; D = 640; H = 32; DH = 20
TQ = 512; NQ = S // TQ
C = 128; NCH = S // C
UPB = 8
NU = NQ * H
VR = 24
F32 = jnp.float32; BF16 = jnp.bfloat16; U32 = jnp.uint32
LOG2E = math.log2(math.e)
QSCALE = (DH ** -0.5) * LOG2E
BOUND_MAX = 30.0
NT = (((1,), (1,)), ((), ()))
TN = (((0,), (0,)), ((), ()))
TP = 512
NH = 4; TH = TQ // NH
LTR = 5 * D + 16
BAND = [((80 * G) // 128, (80 * G + 79) // 128 + 1) for G in range(8)]
R_PQ, R_PK, R_Q, R_VA, R_G, R_VB = 0, D, 2 * D, 3 * D, 4 * D, 4 * D + 16


def _kernel(x_hbm, wa_hbm, woa_hbm, wb_hbm, wphi_hbm, wob_hbm, gate_hbm, out_hbm,
            wphi_ref, gate_ref, x_v, wak_v, waq_v, wav_v, wb_v, wo_v,
            wkt, lt, mscr, tbd, qt, ks, kh, vs, pq_pos, pq_neg, pk_pos, pk_neg, vb, g_row,
            kn, bmx,
            sA, a_even, s0, ot, out_v, sems, osems):
    cp_wk = pltpu.make_async_copy(wa_hbm.at[:, D:2 * D], wak_v, sems.at[0])
    cp_x = [pltpu.make_async_copy(x_hbm.at[pl.ds(i * TP, TP), :], x_v.at[pl.ds(i * TP, TP), :], sems.at[1 + i])
            for i in range(4)]
    cp_wq = pltpu.make_async_copy(wa_hbm.at[:, 0:D], waq_v, sems.at[9])
    cp_wav = pltpu.make_async_copy(wa_hbm.at[:, 2 * D:3 * D], wav_v, sems.at[5])
    cp_wb = pltpu.make_async_copy(wb_hbm, wb_v, sems.at[6])
    cp_woa = pltpu.make_async_copy(woa_hbm, wo_v.at[0:D, :], sems.at[7])
    cp_wob = pltpu.make_async_copy(wob_hbm, wo_v.at[D:2 * D, :], sems.at[8])
    cp_phi = pltpu.make_async_copy(wphi_hbm, wphi_ref, sems.at[10])
    cp_gate = pltpu.make_async_copy(gate_hbm, gate_ref, sems.at[11])
    cp_phi.start()
    cp_wk.start()
    cp_x[0].start()
    cp_gate.start()
    cp_phi.wait()

    for d in range(DH):
        mscr[0:DH, 32 * d: 32 * d + 32] = wphi_ref[d].astype(F32)
    m1 = mscr[0:DH, :].astype(BF16)
    pi = lax.broadcasted_iota(jnp.int32, (D, D), 0)
    pj = lax.broadcasted_iota(jnp.int32, (D, D), 1)
    perm = jnp.where(pj == 20 * (pi & 31) + (pi >> 5), 1.0, 0.0).astype(BF16)
    m2 = jnp.dot(m1, perm, preferred_element_type=F32).astype(BF16)
    ei = lax.broadcasted_iota(jnp.int32, (D, DH), 0)
    ej = lax.broadcasted_iota(jnp.int32, (D, DH), 1)
    et = jnp.where(((ei - 80 * ((ei * 3277) >> 18)) >> 2) == ej, 1.0, 0.0).astype(BF16)
    tiled = jnp.dot(et, m2, preferred_element_type=F32)
    same = (4 * ((pi * 3277) >> 18) + (pi & 3)) == ((pj * 3277) >> 16)
    tbd[...] = jnp.where(same, tiled, 0.0).astype(BF16)

    for cp in cp_x[1:]:
        cp.start()
    cp_wq.start(); cp_wav.start(); cp_wb.start(); cp_woa.start(); cp_wob.start()

    sub = lax.broadcasted_iota(jnp.int32, (16, 8, TP), 1)
    lo = sub < 4

    def pk32(v):
        return pltpu.bitcast(v, U32)

    def up32(v):
        return pltpu.bitcast(v, BF16)

    def tr(w):
        return pk32(w.astype(F32).T.astype(BF16))

    def pairnorm(y):
        y3 = y.reshape(16, 40, TP)
        return jnp.sum(y3 * y3, axis=1, keepdims=True)

    def rev8(a):
        n = a.shape[0]
        return jnp.concatenate([a[128 * b + 8 * (15 - j): 128 * b + 8 * (15 - j) + 8, :]
                                for b in range(n // 128) for j in range(16)], axis=0)

    def ext32(y, fill):
        v3 = y.reshape(16, 40, TP)
        a = [v3[:, 8 * i: 8 * i + 8, :] for i in range(5)]
        z = jnp.zeros((16, 8, TP), F32)
        e2 = jnp.where(lo, a[2], jnp.where(sub == 4, fill, 0.0))
        o0 = jnp.where(lo, jnp.where(sub == 0, fill, 0.0), a[2])
        return jnp.concatenate([a[0], a[1], e2, z, o0, a[3], a[4], z], axis=1)

    def k_proj(tt):
        rows = pl.ds(tt * TP if isinstance(tt, int) else pl.multiple_of(tt * TP, TP), TP)
        hrows = pl.ds(tt * (TP // 2) if isinstance(tt, int) else pl.multiple_of(tt * (TP // 2), TP // 2), TP // 2)
        kt = lax.dot_general(up32(wkt[...]), x_v[rows, :], NT, preferred_element_type=F32)
        ke = ext32(kt, 1.0).reshape(8, 128, TP)
        for G in range(8):
            ks[G, hrows, :] = pk32(rev8(ke[G].T).astype(BF16))
        n = jnp.broadcast_to(pairnorm(kt), (16, 8, TP))
        kn[...] = n if isinstance(tt, int) and tt == 0 else jnp.maximum(kn[...], n)

    def fold(off, row0):
        for j, (k0, k1) in enumerate(BAND):
            r = lax.dot_general(tbd[80 * j: 80 * j + 80, 128 * k0: 128 * k1],
                                wb_v[:, off + 128 * k0: off + 128 * k1], NT, preferred_element_type=F32)
            lt[(row0 + 80 * j) // 2: (row0 + 80 * j + 80) // 2, :] = pk32((r * LOG2E).astype(BF16))

    cp_wk.wait()
    wkt[...] = tr(wak_v[...])
    cp_x[0].wait()
    k_proj(0)
    cp_x[1].wait(); cp_x[2].wait()
    lax.fori_loop(1, 3, lambda tt, c: (k_proj(tt), c)[1], 0)
    cp_x[3].wait(); cp_wq.wait(); cp_wav.wait()
    lt[R_Q // 2:(R_Q + D) // 2, :] = tr(waq_v[...])
    k_proj(3)
    lt[R_VA // 2:(R_VA + D) // 2, :] = tr(wav_v[...])
    cp_wb.wait(); cp_gate.wait()
    fold(0, R_PQ)
    lt[R_VB // 2:(R_VB + D) // 2, :] = tr(wb_v[:, 2 * D:3 * D])
    fold(D, R_PK)
    lt[R_G // 2:(R_G + 16) // 2, :] = pk32(jnp.broadcast_to(gate_ref[...].astype(F32).reshape(1, D), (16, D)).astype(BF16))
    kn[...] = jnp.broadcast_to(jnp.max(kn[...], axis=2, keepdims=True), (16, 8, TP))
    bmx[...] = jnp.zeros_like(bmx)

    def feat(y, pos_ref, neg_ref, cols):
        y4 = y.reshape(8, 10, 8, TP)
        mx = jnp.max(y4, axis=1); mx = jnp.maximum(mx, pltpu.roll(mx, 4, 1))[:, None]
        mn = jnp.min(y4, axis=1); mn = jnp.minimum(mn, pltpu.roll(mn, 4, 1))[:, None]
        for e, ref in ((jnp.exp2(y4 - mx), pos_ref), (jnp.exp2(mn - y4), neg_ref)):
            s = jnp.sum(e, axis=1); s = s + pltpu.roll(s, 4, 1)
            ref[:, cols] = (e * (1.0 / s)[:, None]).reshape(D, TP).astype(BF16)

    def proj(tt, carry):
        cols = pl.ds(pl.multiple_of(tt * TP, TP), TP)
        yt = lax.dot_general(up32(lt[...]), x_v[cols, :], NT, preferred_element_type=F32)
        v3 = yt[R_VA:R_VA + D, :].reshape(16, 40, TP)
        a = [v3[:, 8 * i: 8 * i + 8, :] for i in range(5)]
        e2 = jnp.where(lo, a[2], jnp.where(sub == 4, 1.0, 0.0))
        o0 = jnp.where(lo, jnp.where(sub == 0, 1.0, 0.0), a[2])
        ve = jnp.concatenate([a[0], a[1], e2, o0, a[3], a[4]], axis=1)
        vs[:, :, cols] = ve.reshape(H, VR, TP)
        feat(yt[R_PQ:R_PQ + D, :], pq_pos, pq_neg, cols)
        feat(yt[R_PK:R_PK + D, :], pk_pos, pk_neg, cols)
        vb[:, cols] = yt[R_VB:R_VB + D, :].astype(BF16)
        q = yt[R_Q:R_Q + D, :] * QSCALE
        bnd = jnp.sqrt(pairnorm(q) * kn[...])
        qe = ext32(q, -bnd).reshape(H * 32, TP).astype(BF16)
        qt[:, :, cols] = pk32(qe).reshape(H, 16, TP)
        bmx[...] = jnp.maximum(bmx[...], bnd)
        hrows = pl.ds(pl.multiple_of(tt * (TP // 2), TP // 2), TP // 2)
        for G in range(8):
            t4 = ks[G, hrows, :]
            for jj in range(4):
                kh[4 * G + jj, hrows, :] = t4 if jj == 0 else pltpu.roll(t4, 128 - 32 * jj, 1)
        z = yt[R_G:R_G + 8, :]
        g_row[:, cols] = 1.0 / (1.0 + jnp.exp(-z))
        return carry
    lax.fori_loop(0, S // TP, proj, 0)

    cp_woa.wait()
    cp_wob.wait()
    rr = lax.broadcasted_iota(jnp.int32, (96, 80), 0)
    cc = lax.broadcasted_iota(jnp.int32, (96, 80), 1) & 3
    hrow = jnp.where(rr < 80, (rr * 3277) >> 16, rr - 80)
    bmask = hrow == cc
    lo2 = lax.broadcasted_iota(jnp.int32, (8, S), 0) < 4
    for G in range(8):
        rows = pl.ds(80 * G, 80)
        ones_blk = jnp.where(lax.broadcasted_iota(jnp.int32, (16, S), 0) < 4, 1.0, 0.0).astype(BF16)
        vext = jnp.concatenate([vb[rows, :], ones_blk], axis=0)
        kvp = lax.dot_general(vext, pk_pos[rows, :], NT, preferred_element_type=F32)
        kvn = lax.dot_general(vext, pk_neg[rows, :], NT, preferred_element_type=F32)
        kvp = jnp.where(bmask, kvp, 0.0).astype(BF16)
        kvn = jnp.where(bmask, kvn, 0.0).astype(BF16)
        nd = (jnp.dot(kvp, pq_pos[rows, :], preferred_element_type=F32)
              + jnp.dot(kvn, pq_neg[rows, :], preferred_element_type=F32))
        rden = (1.0 - g_row[0:1, :]) / (nd[80:88, :] + 1e-6)
        for p in range(2):
            rE = rden[2 * p: 2 * p + 1, :]; rO = rden[2 * p + 1: 2 * p + 2, :]
            b0 = 40 * p
            o0 = D + 80 * G + b0
            ot[pl.ds(o0, 16), :] = nd[b0: b0 + 16, :] * rE
            ot[pl.ds(o0 + 16, 8), :] = nd[b0 + 16: b0 + 24, :] * jnp.where(lo2, rE, rO)
            ot[pl.ds(o0 + 24, 16), :] = nd[b0 + 24: b0 + 40, :] * rO

    lo3 = lax.broadcasted_iota(jnp.int32, (8, TQ), 0) < 4

    def qcols(u):
        return pl.ds(pl.multiple_of((u >> 5) * TQ, TQ), TQ)

    def qk_chunk(c, u):
        h = u & 31
        return jnp.dot(up32(kh[h, c * (C // 2):(c + 1) * (C // 2), 0:32]), up32(qt[h, :, qcols(u)]),
                       preferred_element_type=F32)

    def pv_chunk(c, h, p, acc):
        r = jnp.dot(vs[h, :, c * C:(c + 1) * C], rev8(p), preferred_element_type=F32)
        return r if acc is None else acc + r

    def fin(u, acc, odd):
        t = u >> 5; h = u & 31
        cols = pl.ds(pl.multiple_of(t * TQ, TQ), TQ)
        g = g_row[0:1, cols]
        base = pl.multiple_of((h >> 1) * 40, 8)
        if not odd:
            r = g / acc[20:21, :]
            ot[pl.ds(base, 16), cols] = acc[0:16, :] * r
            a_even[...] = acc[16:24, :] * r
        else:
            r = g / acc[0:1, :]
            ot[pl.ds(base + 16, 8), cols] = jnp.where(lo3, a_even[...], acc[0:8, :] * r)
            ot[pl.ds(base + 24, 16), cols] = acc[8:24, :] * r

    safe = jnp.max(bmx[...]) <= BOUND_MAX

    @pl.when(safe)
    def _fast():
        s0[...] = qk_chunk(0, 0)

        def body(j, carry):
            s = s0[...]
            for r in range(UPB):
                u = UPB * j + r
                u1 = jnp.minimum(u + 1, NU - 1)
                acc = None
                for c in range(NCH):
                    s_next = qk_chunk(c + 1, u) if c + 1 < NCH else qk_chunk(0, u1)
                    acc = pv_chunk(c, u & 31, jnp.exp2(s), acc)
                    s = s_next
                fin(u, acc, r % 2 == 1)
            s0[...] = s
            return carry
        lax.fori_loop(0, NU // UPB, body, 0)

    @pl.when(jnp.logical_not(safe))
    def _slow():
        def unit(u, carry):
            h = u & 31
            q = up32(qt[h, :, qcols(u)])
            shift_row = jnp.where((h & 1) == 1, 0, 20)
            q = jnp.where(lax.broadcasted_iota(jnp.int32, (32, TQ), 0) == shift_row, jnp.zeros_like(q), q)

            def p1(c, m8):
                r0 = pl.multiple_of(c * C, C)
                kc = kh[h, pl.ds(pl.multiple_of(c * (C // 2), C // 2), C // 2), 0:32]
                s = jnp.dot(up32(kc), q, preferred_element_type=F32)
                sA[pl.ds(r0, C), :] = s
                return jnp.maximum(m8, jnp.max(s.reshape(C // 8, 8, TQ), axis=0))
            m8 = lax.fori_loop(0, NCH, p1, jnp.full((8, TQ), -jnp.inf, F32))
            m = jnp.max(m8, axis=0, keepdims=True)

            def p2(c, acc):
                r0 = pl.multiple_of(c * C, C)
                p = jnp.exp2(sA[pl.ds(r0, C), :] - m)
                return acc + jnp.dot(vs[h, :, pl.ds(r0, C)], rev8(p), preferred_element_type=F32)
            acc = lax.fori_loop(0, NCH, p2, jnp.zeros((VR, TQ), F32))
            pl.when((u & 1) == 0)(lambda: fin(u, acc, False))
            pl.when((u & 1) == 1)(lambda: fin(u, acc, True))
            return carry
        lax.fori_loop(0, NU, unit, 0)

    def outp(t, carry):
        for hf in range(NH):
            cols = pl.ds(pl.multiple_of(t * TQ + hf * TH, TH), TH)
            o = ot[:, cols].astype(BF16)
            y = lax.dot_general(o, wo_v[...], TN, preferred_element_type=F32)
            out_v[cols, :] = y.astype(BF16)
            pltpu.make_async_copy(out_v.at[cols, :], out_hbm.at[cols, :], osems.at[NH * t + hf]).start()
        return carry
    lax.fori_loop(0, NQ, outp, 0)
    for i in range(NQ * NH):
        rows = pl.ds(i * TH, TH)
        pltpu.make_async_copy(out_v.at[rows, :], out_hbm.at[rows, :], osems.at[i]).wait()


@jax.jit
def pallas_gated_mix__mha_block__linear_kernel_hedgehog__prompt_kernel(
        A_x, A_wqkv, A_wo, B_x, B_wqkv, B_w_phi, B_wo, gate_w):
    x = A_x.reshape(S, D)
    wphi = jnp.transpose(B_w_phi, (1, 2, 0))
    any_spec = pl.BlockSpec(memory_space=pl.ANY)
    out = pl.pallas_call(
        _kernel,
        out_shape=jax.ShapeDtypeStruct((S, D), BF16),
        in_specs=[any_spec] * 7,
        out_specs=any_spec,
        scratch_shapes=[
            pltpu.VMEM((DH, DH, H), BF16), pltpu.VMEM((D,), BF16),
            pltpu.VMEM((S, D), BF16), pltpu.VMEM((D, D), BF16), pltpu.VMEM((D, D), BF16), pltpu.VMEM((D, D), BF16),
            pltpu.VMEM((D, 3 * D), BF16), pltpu.VMEM((2 * D, D), BF16),
            pltpu.VMEM((D // 2, D), U32), pltpu.VMEM((LTR // 2, D), U32),
            pltpu.VMEM((24, D), F32), pltpu.VMEM((D, D), BF16),
            pltpu.VMEM((H, 16, S), U32), pltpu.VMEM((8, S // 2, 128), U32), pltpu.VMEM((H, S // 2, 128), U32), pltpu.VMEM((H, VR, S), F32),
            pltpu.VMEM((D, S), BF16), pltpu.VMEM((D, S), BF16), pltpu.VMEM((D, S), BF16), pltpu.VMEM((D, S), BF16),
            pltpu.VMEM((D, S), BF16), pltpu.VMEM((8, S), F32),
            pltpu.VMEM((16, 8, TP), F32), pltpu.VMEM((16, 8, TP), F32),
            pltpu.VMEM((S, TQ), F32), pltpu.VMEM((8, TQ), F32),
            pltpu.VMEM((C, TQ), F32),
            pltpu.VMEM((2 * D, S), F32), pltpu.VMEM((S, D), BF16),
            pltpu.SemaphoreType.DMA((12,)), pltpu.SemaphoreType.DMA((NQ * NH,)),
        ],
        compiler_params=pltpu.CompilerParams(vmem_limit_bytes=110 * 1024 * 1024),
    )(x, A_wqkv, A_wo, B_wqkv, wphi, B_wo, gate_w)
    return out.reshape(1, S, D)
```

```python
import math

import jax
import jax.numpy as jnp
from jax import lax
from jax.experimental import pallas as pl
from jax.experimental.pallas import tpu as pltpu

S = 2048; D = 640; H = 32; DH = 20
TQ = 512; NQ = S // TQ
C = 128; NCH = S // C
UPB = 8
NU = NQ * H
VR = 24
F32 = jnp.float32; BF16 = jnp.bfloat16; U32 = jnp.uint32
LOG2E = math.log2(math.e)
QSCALE = (DH ** -0.5) * LOG2E
BOUND_MAX = 30.0
NT = (((1,), (1,)), ((), ()))
TN = (((0,), (0,)), ((), ()))
TP = 512
NH = 4; TH = TQ // NH
LTR = 5 * D + 16
BAND = [((80 * G) // 128, (80 * G + 79) // 128 + 1) for G in range(8)]
R_PQ, R_PK, R_Q, R_VA, R_G, R_VB = 0, D, 2 * D, 3 * D, 4 * D, 4 * D + 16


def _kernel(x_hbm, wa_hbm, woa_hbm, wb_hbm, wphi_hbm, wob_hbm, gate_hbm, out_hbm,
            wphi_ref, gate_ref, x_v, wak_v, waq_v, wav_v, wb_v, wo_v,
            wkt, lt, mscr, tbd, qt, ks, kh, vs, pq_pos, pq_neg, pk_pos, pk_neg, vb, g_row,
            kn, bmx,
            sA, a_even, a_last, s0, ot, out_v, sems, osems):
    cp_wk = pltpu.make_async_copy(wa_hbm.at[:, D:2 * D], wak_v, sems.at[0])
    cp_x = [pltpu.make_async_copy(x_hbm.at[pl.ds(i * TP, TP), :], x_v.at[pl.ds(i * TP, TP), :], sems.at[1 + i])
            for i in range(4)]
    cp_wq = pltpu.make_async_copy(wa_hbm.at[:, 0:D], waq_v, sems.at[9])
    cp_wav = pltpu.make_async_copy(wa_hbm.at[:, 2 * D:3 * D], wav_v, sems.at[5])
    cp_wb = pltpu.make_async_copy(wb_hbm, wb_v, sems.at[6])
    cp_woa = pltpu.make_async_copy(woa_hbm, wo_v.at[0:D, :], sems.at[7])
    cp_wob = pltpu.make_async_copy(wob_hbm, wo_v.at[D:2 * D, :], sems.at[8])
    cp_phi = pltpu.make_async_copy(wphi_hbm, wphi_ref, sems.at[10])
    cp_gate = pltpu.make_async_copy(gate_hbm, gate_ref, sems.at[11])
    cp_phi.start()
    cp_wk.start()
    cp_x[0].start()
    cp_gate.start()
    cp_phi.wait()

    for d in range(DH):
        mscr[0:DH, 32 * d: 32 * d + 32] = wphi_ref[d].astype(F32)
    m1 = mscr[0:DH, :].astype(BF16)
    pi = lax.broadcasted_iota(jnp.int32, (D, D), 0)
    pj = lax.broadcasted_iota(jnp.int32, (D, D), 1)
    perm = jnp.where(pj == 20 * (pi & 31) + (pi >> 5), 1.0, 0.0).astype(BF16)
    m2 = jnp.dot(m1, perm, preferred_element_type=F32).astype(BF16)
    ei = lax.broadcasted_iota(jnp.int32, (D, DH), 0)
    ej = lax.broadcasted_iota(jnp.int32, (D, DH), 1)
    et = jnp.where(((ei - 80 * ((ei * 3277) >> 18)) >> 2) == ej, 1.0, 0.0).astype(BF16)
    tiled = jnp.dot(et, m2, preferred_element_type=F32)
    same = (4 * ((pi * 3277) >> 18) + (pi & 3)) == ((pj * 3277) >> 16)
    tbd[...] = jnp.where(same, tiled, 0.0).astype(BF16)

    for cp in cp_x[1:]:
        cp.start()
    cp_wq.start(); cp_wav.start(); cp_wb.start(); cp_woa.start(); cp_wob.start()

    sub = lax.broadcasted_iota(jnp.int32, (16, 8, TP), 1)
    lo = sub < 4

    def pk32(v):
        return pltpu.bitcast(v, U32)

    def up32(v):
        return pltpu.bitcast(v, BF16)

    def tr(w):
        return pk32(w.astype(F32).T.astype(BF16))

    def pairnorm(y):
        y3 = y.reshape(16, 40, TP)
        return jnp.sum(y3 * y3, axis=1, keepdims=True)

    def rev8(a):
        n = a.shape[0]
        return jnp.concatenate([a[128 * b + 8 * (15 - j): 128 * b + 8 * (15 - j) + 8, :]
                                for b in range(n // 128) for j in range(16)], axis=0)

    def ext32(y, fill):
        v3 = y.reshape(16, 40, TP)
        a = [v3[:, 8 * i: 8 * i + 8, :] for i in range(5)]
        z = jnp.zeros((16, 8, TP), F32)
        e2 = jnp.where(lo, a[2], jnp.where(sub == 4, fill, 0.0))
        o0 = jnp.where(lo, jnp.where(sub == 0, fill, 0.0), a[2])
        return jnp.concatenate([a[0], a[1], e2, z, o0, a[3], a[4], z], axis=1)

    def k_proj(tt):
        rows = pl.ds(tt * TP if isinstance(tt, int) else pl.multiple_of(tt * TP, TP), TP)
        hrows = pl.ds(tt * (TP // 2) if isinstance(tt, int) else pl.multiple_of(tt * (TP // 2), TP // 2), TP // 2)
        kt = lax.dot_general(up32(wkt[...]), x_v[rows, :], NT, preferred_element_type=F32)
        ke = ext32(kt, 1.0).reshape(8, 128, TP)
        for G in range(8):
            ks[G, hrows, :] = pk32(rev8(ke[G].T).astype(BF16))
        n = jnp.broadcast_to(pairnorm(kt), (16, 8, TP))
        kn[...] = n if isinstance(tt, int) and tt == 0 else jnp.maximum(kn[...], n)

    def fold(off, row0):
        for j, (k0, k1) in enumerate(BAND):
            r = lax.dot_general(tbd[80 * j: 80 * j + 80, 128 * k0: 128 * k1],
                                wb_v[:, off + 128 * k0: off + 128 * k1], NT, preferred_element_type=F32)
            lt[(row0 + 80 * j) // 2: (row0 + 80 * j + 80) // 2, :] = pk32((r * LOG2E).astype(BF16))

    cp_wk.wait()
    wkt[...] = tr(wak_v[...])
    cp_x[0].wait()
    k_proj(0)
    cp_x[1].wait(); cp_x[2].wait()
    lax.fori_loop(1, 3, lambda tt, c: (k_proj(tt), c)[1], 0)
    cp_x[3].wait(); cp_wq.wait(); cp_wav.wait()
    lt[R_Q // 2:(R_Q + D) // 2, :] = tr(waq_v[...])
    k_proj(3)
    lt[R_VA // 2:(R_VA + D) // 2, :] = tr(wav_v[...])
    cp_wb.wait(); cp_gate.wait()
    fold(0, R_PQ)
    lt[R_VB // 2:(R_VB + D) // 2, :] = tr(wb_v[:, 2 * D:3 * D])
    fold(D, R_PK)
    lt[R_G // 2:(R_G + 16) // 2, :] = pk32(jnp.broadcast_to(gate_ref[...].astype(F32).reshape(1, D), (16, D)).astype(BF16))
    kn[...] = jnp.broadcast_to(jnp.max(kn[...], axis=2, keepdims=True), (16, 8, TP))
    bmx[...] = jnp.zeros_like(bmx)

    def feat(y, pos_ref, neg_ref, cols):
        y4 = y.reshape(8, 10, 8, TP)
        mx = jnp.max(y4, axis=1); mx = jnp.maximum(mx, pltpu.roll(mx, 4, 1))[:, None]
        mn = jnp.min(y4, axis=1); mn = jnp.minimum(mn, pltpu.roll(mn, 4, 1))[:, None]
        for e, ref in ((jnp.exp2(y4 - mx), pos_ref), (jnp.exp2(mn - y4), neg_ref)):
            s = jnp.sum(e, axis=1); s = s + pltpu.roll(s, 4, 1)
            ref[:, cols] = (e * (1.0 / s)[:, None]).reshape(D, TP)

    def proj(tt, carry):
        cols = pl.ds(pl.multiple_of(tt * TP, TP), TP)
        yt = lax.dot_general(up32(lt[...]), x_v[cols, :], NT, preferred_element_type=F32)
        v3 = yt[R_VA:R_VA + D, :].reshape(16, 40, TP)
        a = [v3[:, 8 * i: 8 * i + 8, :] for i in range(5)]
        e2 = jnp.where(lo, a[2], jnp.where(sub == 4, 1.0, 0.0))
        o0 = jnp.where(lo, jnp.where(sub == 0, 1.0, 0.0), a[2])
        ve = jnp.concatenate([a[0], a[1], e2, o0, a[3], a[4]], axis=1)
        vs[:, :, cols] = ve.reshape(H, VR, TP)
        feat(yt[R_PQ:R_PQ + D, :], pq_pos, pq_neg, cols)
        feat(yt[R_PK:R_PK + D, :], pk_pos, pk_neg, cols)
        vb[:, cols] = yt[R_VB:R_VB + D, :]
        q = yt[R_Q:R_Q + D, :] * QSCALE
        bnd = jnp.sqrt(pairnorm(q) * kn[...])
        qe = ext32(q, -bnd).reshape(H * 32, TP).astype(BF16)
        qt[:, :, cols] = pk32(qe).reshape(H, 16, TP)
        bmx[...] = jnp.maximum(bmx[...], bnd)
        hrows = pl.ds(pl.multiple_of(tt * (TP // 2), TP // 2), TP // 2)
        for G in range(8):
            t4 = ks[G, hrows, :]
            for jj in range(4):
                kh[4 * G + jj, hrows, :] = t4 if jj == 0 else pltpu.roll(t4, 128 - 32 * jj, 1)
        z = yt[R_G:R_G + 8, :]
        g_row[:, cols] = 1.0 / (1.0 + jnp.exp(-z))
        return carry
    lax.fori_loop(0, S // TP, proj, 0)

    cp_woa.wait()
    cp_wob.wait()
    rr = lax.broadcasted_iota(jnp.int32, (88, 80), 0)
    cc = lax.broadcasted_iota(jnp.int32, (88, 80), 1) & 3
    hrow = jnp.where(rr < 80, (rr * 3277) >> 16, rr - 80)
    bmask = hrow == cc
    lo2 = lax.broadcasted_iota(jnp.int32, (8, S), 0) < 4
    for G in range(8):
        rows = pl.ds(80 * G, 80)
        ones_blk = jnp.where(lax.broadcasted_iota(jnp.int32, (8, S), 0) < 4, 1.0, 0.0)
        vext = jnp.concatenate([vb[rows, :], ones_blk], axis=0)
        kvp = lax.dot_general(vext, pk_pos[rows, :], NT, preferred_element_type=F32)
        kvn = lax.dot_general(vext, pk_neg[rows, :], NT, preferred_element_type=F32)
        kvp = jnp.where(bmask, kvp, 0.0)
        kvn = jnp.where(bmask, kvn, 0.0)
        nd = (jnp.dot(kvp, pq_pos[rows, :], preferred_element_type=F32)
              + jnp.dot(kvn, pq_neg[rows, :], preferred_element_type=F32))
        rden = (1.0 - g_row[0:1, :]) / (nd[80:88, :] + 1e-6)
        for p in range(2):
            rE = rden[2 * p: 2 * p + 1, :]; rO = rden[2 * p + 1: 2 * p + 2, :]
            b0 = 40 * p
            o0 = D + 80 * G + b0
            ot[pl.ds(o0, 16), :] = nd[b0: b0 + 16, :] * rE
            ot[pl.ds(o0 + 16, 8), :] = nd[b0 + 16: b0 + 24, :] * jnp.where(lo2, rE, rO)
            ot[pl.ds(o0 + 24, 16), :] = nd[b0 + 24: b0 + 40, :] * rO

    lo3 = lax.broadcasted_iota(jnp.int32, (8, TQ), 0) < 4

    def qcols(u):
        return pl.ds(pl.multiple_of((u >> 5) * TQ, TQ), TQ)

    def qk_chunk(c, u):
        h = u & 31
        return jnp.dot(up32(kh[h, c * (C // 2):(c + 1) * (C // 2), 0:32]), up32(qt[h, :, qcols(u)]),
                       preferred_element_type=F32)

    def pv_chunk(c, h, p, acc):
        r = jnp.dot(vs[h, :, c * C:(c + 1) * C], rev8(p), preferred_element_type=F32)
        return r if acc is None else acc + r

    def fin(u, acc, odd):
        t = u >> 5; h = u & 31
        cols = pl.ds(pl.multiple_of(t * TQ, TQ), TQ)
        g = g_row[0:1, cols]
        base = pl.multiple_of((h >> 1) * 40, 8)
        if not odd:
            r = g / acc[20:21, :]
            ot[pl.ds(base, 16), cols] = acc[0:16, :] * r
            a_even[...] = acc[16:24, :] * r
        else:
            r = g / acc[0:1, :]
            ot[pl.ds(base + 16, 8), cols] = jnp.where(lo3, a_even[...], acc[0:8, :] * r)
            ot[pl.ds(base + 24, 16), cols] = acc[8:24, :] * r

    safe = jnp.max(bmx[...]) <= BOUND_MAX

    @pl.when(safe)
    def _fast():
        s0[...] = qk_chunk(0, 0)
        a_last[...] = jnp.ones_like(a_last)
        a_even[...] = jnp.zeros_like(a_even)

        def body(j, carry):
            s = s0[...]
            for r in range(UPB):
                u = UPB * j + r
                u1 = jnp.minimum(u + 1, NU - 1)
                acc = None
                for c in range(NCH):
                    s_next = qk_chunk(c + 1, u) if c + 1 < NCH else qk_chunk(0, u1)
                    acc = pv_chunk(c, u & 31, jnp.exp2(s), acc)
                    s = s_next
                    if r == 0 and c == 3:
                        fin(jnp.maximum(u - 1, 1), a_last[...], True)
                if r < UPB - 1:
                    fin(u, acc, r % 2 == 1)
                else:
                    a_last[...] = acc
            s0[...] = s
            return carry
        lax.fori_loop(0, NU // UPB, body, 0)
        fin(NU - 1, a_last[...], True)

    @pl.when(jnp.logical_not(safe))
    def _slow():
        def unit(u, carry):
            h = u & 31
            q = up32(qt[h, :, qcols(u)])
            shift_row = jnp.where((h & 1) == 1, 0, 20)
            q = jnp.where(lax.broadcasted_iota(jnp.int32, (32, TQ), 0) == shift_row, jnp.zeros_like(q), q)

            def p1(c, m8):
                r0 = pl.multiple_of(c * C, C)
                kc = kh[h, pl.ds(pl.multiple_of(c * (C // 2), C // 2), C // 2), 0:32]
                s = jnp.dot(up32(kc), q, preferred_element_type=F32)
                sA[pl.ds(r0, C), :] = s
                return jnp.maximum(m8, jnp.max(s.reshape(C // 8, 8, TQ), axis=0))
            m8 = lax.fori_loop(0, NCH, p1, jnp.full((8, TQ), -jnp.inf, F32))
            m = jnp.max(m8, axis=0, keepdims=True)

            def p2(c, acc):
                r0 = pl.multiple_of(c * C, C)
                p = jnp.exp2(sA[pl.ds(r0, C), :] - m)
                return acc + jnp.dot(vs[h, :, pl.ds(r0, C)], rev8(p), preferred_element_type=F32)
            acc = lax.fori_loop(0, NCH, p2, jnp.zeros((VR, TQ), F32))
            pl.when((u & 1) == 0)(lambda: fin(u, acc, False))
            pl.when((u & 1) == 1)(lambda: fin(u, acc, True))
            return carry
        lax.fori_loop(0, NU, unit, 0)

    def outp(t, carry):
        for hf in range(NH):
            cols = pl.ds(pl.multiple_of(t * TQ + hf * TH, TH), TH)
            o = ot[:, cols].T.astype(BF16)
            y = jnp.dot(o, wo_v[...], preferred_element_type=F32)
            out_v[cols, :] = y.astype(BF16)
            pltpu.make_async_copy(out_v.at[cols, :], out_hbm.at[cols, :], osems.at[NH * t + hf]).start()
        return carry
    lax.fori_loop(0, NQ, outp, 0)
    for i in range(NQ * NH):
        rows = pl.ds(i * TH, TH)
        pltpu.make_async_copy(out_v.at[rows, :], out_hbm.at[rows, :], osems.at[i]).wait()


@jax.jit
def pallas_gated_mix__mha_block__linear_kernel_hedgehog__prompt_kernel(
        A_x, A_wqkv, A_wo, B_x, B_wqkv, B_w_phi, B_wo, gate_w):
    x = A_x.reshape(S, D)
    wphi = jnp.transpose(B_w_phi, (1, 2, 0))
    any_spec = pl.BlockSpec(memory_space=pl.ANY)
    out = pl.pallas_call(
        _kernel,
        out_shape=jax.ShapeDtypeStruct((S, D), BF16),
        in_specs=[any_spec] * 7,
        out_specs=any_spec,
        scratch_shapes=[
            pltpu.VMEM((DH, DH, H), BF16), pltpu.VMEM((D,), BF16),
            pltpu.VMEM((S, D), BF16), pltpu.VMEM((D, D), BF16), pltpu.VMEM((D, D), BF16), pltpu.VMEM((D, D), BF16),
            pltpu.VMEM((D, 3 * D), BF16), pltpu.VMEM((2 * D, D), BF16),
            pltpu.VMEM((D // 2, D), U32), pltpu.VMEM((LTR // 2, D), U32),
            pltpu.VMEM((24, D), F32), pltpu.VMEM((D, D), BF16),
            pltpu.VMEM((H, 16, S), U32), pltpu.VMEM((8, S // 2, 128), U32), pltpu.VMEM((H, S // 2, 128), U32), pltpu.VMEM((H, VR, S), F32),
            pltpu.VMEM((D, S), F32), pltpu.VMEM((D, S), F32), pltpu.VMEM((D, S), F32), pltpu.VMEM((D, S), F32),
            pltpu.VMEM((D, S), F32), pltpu.VMEM((8, S), F32),
            pltpu.VMEM((16, 8, TP), F32), pltpu.VMEM((16, 8, TP), F32),
            pltpu.VMEM((S, TQ), F32), pltpu.VMEM((8, TQ), F32), pltpu.VMEM((VR, TQ), F32),
            pltpu.VMEM((C, TQ), F32),
            pltpu.VMEM((2 * D, S), F32), pltpu.VMEM((S, D), BF16),
            pltpu.SemaphoreType.DMA((12,)), pltpu.SemaphoreType.DMA((NQ * NH,)),
        ],
        compiler_params=pltpu.CompilerParams(vmem_limit_bytes=110 * 1024 * 1024),
    )(x, A_wqkv, A_wo, B_wqkv, wphi, B_wo, gate_w)
    return out.reshape(1, S, D)
```

```python
import math

import jax
import jax.numpy as jnp
from jax import lax
from jax.experimental import pallas as pl
from jax.experimental.pallas import tpu as pltpu

S = 2048; D = 640; H = 32; DH = 20
TQ = 512; NQ = S // TQ
C = 128; NCH = S // C
UPB = 8
NU = NQ * H
VR = 24
F32 = jnp.float32; BF16 = jnp.bfloat16; U32 = jnp.uint32
LOG2E = math.log2(math.e)
QSCALE = (DH ** -0.5) * LOG2E
BOUND_MAX = 30.0
NT = (((1,), (1,)), ((), ()))
TN = (((0,), (0,)), ((), ()))
TP = 512
NH = 4; TH = TQ // NH
LTR = 5 * D + 16
BAND = [((80 * G) // 128, (80 * G + 79) // 128 + 1) for G in range(8)]
KB = (1, 2, 2)
R_PQ, R_PK, R_Q, R_VA, R_G, R_VB = 0, D, 2 * D, 3 * D, 4 * D, 4 * D + 16


def _kernel(x_hbm, wa_hbm, woa_hbm, wb_hbm, wphi_hbm, wob_hbm, gate_hbm, out_hbm,
            wphi_ref, gate_ref, x_v, wak_v, waq_v, wav_v, wb_v, wo_v,
            wkt, lt, mscr, tbd, qt, ks, kh, vs, pq_pos, pq_neg, pk_pos, pk_neg, vb, g_row,
            kn, bmx,
            sA, a_even, a_last, s0, ot, out_v, kacc, sems, osems):
    cp_x = [None] + [pltpu.make_async_copy(x_hbm.at[pl.ds(i * TP, TP), :], x_v.at[pl.ds(i * TP, TP), :], sems.at[1 + i])
                     for i in range(1, 4)]
    cp_wq = pltpu.make_async_copy(wa_hbm.at[:, 0:D], waq_v, sems.at[9])
    cp_wav = pltpu.make_async_copy(wa_hbm.at[:, 2 * D:3 * D], wav_v, sems.at[5])
    cp_wb = pltpu.make_async_copy(wb_hbm, wb_v, sems.at[6])
    cp_woa = pltpu.make_async_copy(woa_hbm, wo_v.at[0:D, :], sems.at[7])
    cp_wob = pltpu.make_async_copy(wob_hbm, wo_v.at[D:2 * D, :], sems.at[8])
    cp_phi = pltpu.make_async_copy(wphi_hbm, wphi_ref, sems.at[10])
    cp_gate = pltpu.make_async_copy(gate_hbm, gate_ref, sems.at[11])
    kb0 = [128 * sum(KB[:i]) for i in range(len(KB))]
    cp_wkp = [pltpu.make_async_copy(wa_hbm.at[pl.ds(kb0[i], 128 * KB[i]), pl.ds(D, D)],
                                    wak_v.at[pl.ds(kb0[i], 128 * KB[i]), :], sems.at[12 + i]) for i in range(len(KB))]
    cp_x0p = [pltpu.make_async_copy(x_hbm.at[pl.ds(0, TP), pl.ds(kb0[i], 128 * KB[i])],
                                    x_v.at[pl.ds(0, TP), pl.ds(kb0[i], 128 * KB[i])], sems.at[15 + i]) for i in range(len(KB))]
    cp_phi.start()
    for i in range(len(KB)):
        cp_wkp[i].start()
        cp_x0p[i].start()
    cp_gate.start()
    cp_phi.wait()

    for d in range(DH):
        mscr[0:DH, 32 * d: 32 * d + 32] = wphi_ref[d].astype(F32)
    m1 = mscr[0:DH, :].astype(BF16)
    pi = lax.broadcasted_iota(jnp.int32, (D, D), 0)
    pj = lax.broadcasted_iota(jnp.int32, (D, D), 1)
    perm = jnp.where(pj == 20 * (pi & 31) + (pi >> 5), 1.0, 0.0).astype(BF16)
    m2 = jnp.dot(m1, perm, preferred_element_type=F32).astype(BF16)
    ei = lax.broadcasted_iota(jnp.int32, (80, DH), 0)
    ej = lax.broadcasted_iota(jnp.int32, (80, DH), 1)
    et = jnp.where((ei >> 2) == ej, 1.0, 0.0).astype(BF16)
    for G, (k0, k1) in enumerate(BAND):
        cw = 128 * (k1 - k0)
        tiled = jnp.dot(et, m2[:, 128 * k0: 128 * k1], preferred_element_type=F32)
        ri = lax.broadcasted_iota(jnp.int32, (80, cw), 0)
        ci = lax.broadcasted_iota(jnp.int32, (80, cw), 1) + 128 * k0
        same = (4 * G + (ri & 3)) == ((ci * 3277) >> 16)
        tbd[G, :, 0:cw] = jnp.where(same, tiled, 0.0).astype(BF16)

    for cp in cp_x[1:]:
        cp.start()
    cp_wq.start(); cp_wav.start(); cp_wb.start(); cp_woa.start(); cp_wob.start()

    sub = lax.broadcasted_iota(jnp.int32, (16, 8, TP), 1)
    lo = sub < 4

    def pk32(v):
        return pltpu.bitcast(v, U32)

    def up32(v):
        return pltpu.bitcast(v, BF16)

    def tr(w):
        return pk32(w.astype(F32).T.astype(BF16))

    def pairnorm(y):
        y3 = y.reshape(16, 40, TP)
        return jnp.sum(y3 * y3, axis=1, keepdims=True)

    def rev8(a):
        n = a.shape[0]
        return jnp.concatenate([a[128 * b + 8 * (15 - j): 128 * b + 8 * (15 - j) + 8, :]
                                for b in range(n // 128) for j in range(16)], axis=0)

    def ext32(y, fill):
        v3 = y.reshape(16, 40, TP)
        a = [v3[:, 8 * i: 8 * i + 8, :] for i in range(5)]
        z = jnp.zeros((16, 8, TP), F32)
        e2 = jnp.where(lo, a[2], jnp.where(sub == 4, fill, 0.0))
        o0 = jnp.where(lo, jnp.where(sub == 0, fill, 0.0), a[2])
        return jnp.concatenate([a[0], a[1], e2, z, o0, a[3], a[4], z], axis=1)

    def k_proj(tt, kt=None):
        rows = pl.ds(tt * TP if isinstance(tt, int) else pl.multiple_of(tt * TP, TP), TP)
        hrows = pl.ds(tt * (TP // 2) if isinstance(tt, int) else pl.multiple_of(tt * (TP // 2), TP // 2), TP // 2)
        if kt is None:
            kt = lax.dot_general(up32(wkt[...]), x_v[rows, :], NT, preferred_element_type=F32)
        ke = ext32(kt, 1.0).reshape(8, 128, TP)
        for G in range(8):
            ks[G, hrows, :] = pk32(rev8(ke[G].T).astype(BF16))
        n = jnp.broadcast_to(pairnorm(kt), (16, 8, TP))
        kn[...] = n if isinstance(tt, int) and tt == 0 else jnp.maximum(kn[...], n)

    def fold(off, row0):
        for j, (k0, k1) in enumerate(BAND):
            r = lax.dot_general(tbd[j, :, 0:128 * (k1 - k0)],
                                wb_v[:, off + 128 * k0: off + 128 * k1], NT, preferred_element_type=F32)
            lt[(row0 + 80 * j) // 2: (row0 + 80 * j + 80) // 2, :] = pk32((r * LOG2E).astype(BF16))

    for i in range(len(KB)):
        c0 = kb0[i]; cw = 128 * KB[i]
        cp_wkp[i].wait(); cp_x0p[i].wait()
        wt = tr(wak_v[c0:c0 + cw, :])
        wkt[:, c0:c0 + cw] = wt
        part = lax.dot_general(up32(wt), x_v[0:TP, c0:c0 + cw], NT, preferred_element_type=F32)
        if i > 0:
            part = part + kacc[...]
        if i < len(KB) - 1:
            kacc[...] = part
        else:
            k_proj(0, part)
    def k_step(tt, carry):
        rows = pl.ds(pl.multiple_of(tt * TP, TP), TP)
        pltpu.make_async_copy(x_hbm.at[rows, :], x_v.at[rows, :], sems.at[1 + tt]).wait()
        k_proj(tt)
        return carry
    lax.fori_loop(1, 3, k_step, 0)
    cp_x[3].wait(); cp_wq.wait(); cp_wav.wait()
    lt[R_Q // 2:(R_Q + D) // 2, :] = tr(waq_v[...])
    k_proj(3)
    lt[R_VA // 2:(R_VA + D) // 2, :] = tr(wav_v[...])
    cp_wb.wait(); cp_gate.wait()
    fold(0, R_PQ)
    lt[R_VB // 2:(R_VB + D) // 2, :] = tr(wb_v[:, 2 * D:3 * D])
    fold(D, R_PK)
    lt[R_G // 2:(R_G + 16) // 2, :] = pk32(jnp.broadcast_to(gate_ref[...].astype(F32).reshape(1, D), (16, D)).astype(BF16))
    kn[...] = jnp.broadcast_to(jnp.max(kn[...], axis=2, keepdims=True), (16, 8, TP))
    bmx[...] = jnp.zeros_like(bmx)

    def feat(y, pos_ref, neg_ref, cols):
        y4 = y.reshape(8, 10, 8, TP)
        mx = jnp.max(y4, axis=1); mx = jnp.maximum(mx, pltpu.roll(mx, 4, 1))[:, None]
        mn = jnp.min(y4, axis=1); mn = jnp.minimum(mn, pltpu.roll(mn, 4, 1))[:, None]
        for e, ref in ((jnp.exp2(y4 - mx), pos_ref), (jnp.exp2(mn - y4), neg_ref)):
            s = jnp.sum(e, axis=1); s = s + pltpu.roll(s, 4, 1)
            ref[:, cols] = (e * (1.0 / s)[:, None]).reshape(D, TP)

    def proj(tt, carry):
        cols = pl.ds(pl.multiple_of(tt * TP, TP), TP)
        yt = lax.dot_general(up32(lt[...]), x_v[cols, :], NT, preferred_element_type=F32)
        v3 = yt[R_VA:R_VA + D, :].reshape(16, 40, TP)
        a = [v3[:, 8 * i: 8 * i + 8, :] for i in range(5)]
        e2 = jnp.where(lo, a[2], jnp.where(sub == 4, 1.0, 0.0))
        o0 = jnp.where(lo, jnp.where(sub == 0, 1.0, 0.0), a[2])
        ve = jnp.concatenate([a[0], a[1], e2, o0, a[3], a[4]], axis=1)
        vs[:, :, cols] = ve.reshape(H, VR, TP)
        feat(yt[R_PQ:R_PQ + D, :], pq_pos, pq_neg, cols)
        feat(yt[R_PK:R_PK + D, :], pk_pos, pk_neg, cols)
        vb[:, cols] = yt[R_VB:R_VB + D, :]
        q = yt[R_Q:R_Q + D, :] * QSCALE
        bnd = jnp.sqrt(pairnorm(q) * kn[...])
        qe = ext32(q, -bnd).reshape(H * 32, TP).astype(BF16)
        qt[:, :, cols] = pk32(qe).reshape(H, 16, TP)
        bmx[...] = jnp.maximum(bmx[...], bnd)
        hrows = pl.ds(pl.multiple_of(tt * (TP // 2), TP // 2), TP // 2)
        for G in range(8):
            t4 = ks[G, hrows, :]
            for jj in range(4):
                kh[4 * G + jj, hrows, :] = t4 if jj == 0 else pltpu.roll(t4, 128 - 32 * jj, 1)
        z = yt[R_G:R_G + 8, :]
        g_row[:, cols] = 1.0 / (1.0 + jnp.exp(-z))
        return carry
    lax.fori_loop(0, S // TP, proj, 0)

    cp_woa.wait()
    cp_wob.wait()
    rr = lax.broadcasted_iota(jnp.int32, (88, 80), 0)
    cc = lax.broadcasted_iota(jnp.int32, (88, 80), 1) & 3
    hrow = jnp.where(rr < 80, (rr * 3277) >> 16, rr - 80)
    bmask = hrow == cc
    lo2 = lax.broadcasted_iota(jnp.int32, (8, S), 0) < 4
    for G in range(8):
        rows = pl.ds(80 * G, 80)
        ones_blk = jnp.where(lax.broadcasted_iota(jnp.int32, (8, S), 0) < 4, 1.0, 0.0)
        vext = jnp.concatenate([vb[rows, :], ones_blk], axis=0)
        kvp = lax.dot_general(vext, pk_pos[rows, :], NT, preferred_element_type=F32)
        kvn = lax.dot_general(vext, pk_neg[rows, :], NT, preferred_element_type=F32)
        kvp = jnp.where(bmask, kvp, 0.0)
        kvn = jnp.where(bmask, kvn, 0.0)
        nd = (jnp.dot(kvp, pq_pos[rows, :], preferred_element_type=F32)
              + jnp.dot(kvn, pq_neg[rows, :], preferred_element_type=F32))
        rden = (1.0 - g_row[0:1, :]) / (nd[80:88, :] + 1e-6)
        for p in range(2):
            rE = rden[2 * p: 2 * p + 1, :]; rO = rden[2 * p + 1: 2 * p + 2, :]
            b0 = 40 * p
            o0 = D + 80 * G + b0
            ot[pl.ds(o0, 16), :] = nd[b0: b0 + 16, :] * rE
            ot[pl.ds(o0 + 16, 8), :] = nd[b0 + 16: b0 + 24, :] * jnp.where(lo2, rE, rO)
            ot[pl.ds(o0 + 24, 16), :] = nd[b0 + 24: b0 + 40, :] * rO

    lo3 = lax.broadcasted_iota(jnp.int32, (8, TQ), 0) < 4

    def qcols(u):
        return pl.ds(pl.multiple_of((u >> 5) * TQ, TQ), TQ)

    def qk_chunk(c, u):
        h = u & 31
        return jnp.dot(up32(kh[h, c * (C // 2):(c + 1) * (C // 2), 0:32]), up32(qt[h, :, qcols(u)]),
                       preferred_element_type=F32)

    def pv_chunk(c, h, p, acc):
        r = jnp.dot(vs[h, :, c * C:(c + 1) * C], rev8(p), preferred_element_type=F32)
        return r if acc is None else acc + r

    def fin(u, acc, odd):
        t = u >> 5; h = u & 31
        cols = pl.ds(pl.multiple_of(t * TQ, TQ), TQ)
        g = g_row[0:1, cols]
        base = pl.multiple_of((h >> 1) * 40, 8)
        if not odd:
            r = g / acc[20:21, :]
            ot[pl.ds(base, 16), cols] = acc[0:16, :] * r
            a_even[...] = acc[16:24, :] * r
        else:
            r = g / acc[0:1, :]
            ot[pl.ds(base + 16, 8), cols] = jnp.where(lo3, a_even[...], acc[0:8, :] * r)
            ot[pl.ds(base + 24, 16), cols] = acc[8:24, :] * r

    safe = jnp.max(bmx[...]) <= BOUND_MAX

    @pl.when(safe)
    def _fast():
        s0[...] = qk_chunk(0, 0)
        a_last[...] = jnp.ones_like(a_last)
        a_even[...] = jnp.zeros_like(a_even)

        def body(j, carry):
            s = s0[...]
            for r in range(UPB):
                u = UPB * j + r
                u1 = jnp.minimum(u + 1, NU - 1)
                acc = None
                for c in range(NCH):
                    s_next = qk_chunk(c + 1, u) if c + 1 < NCH else qk_chunk(0, u1)
                    acc = pv_chunk(c, u & 31, jnp.exp2(s), acc)
                    s = s_next
                    if r == 0 and c == 3:
                        fin(jnp.maximum(u - 1, 1), a_last[...], True)
                if r < UPB - 1:
                    fin(u, acc, r % 2 == 1)
                else:
                    a_last[...] = acc
            s0[...] = s
            return carry
        lax.fori_loop(0, NU // UPB, body, 0)
        fin(NU - 1, a_last[...], True)

    @pl.when(jnp.logical_not(safe))
    def _slow():
        def unit(u, carry):
            h = u & 31
            q = up32(qt[h, :, qcols(u)])
            shift_row = jnp.where((h & 1) == 1, 0, 20)
            q = jnp.where(lax.broadcasted_iota(jnp.int32, (32, TQ), 0) == shift_row, jnp.zeros_like(q), q)

            def p1(c, m8):
                r0 = pl.multiple_of(c * C, C)
                kc = kh[h, pl.ds(pl.multiple_of(c * (C // 2), C // 2), C // 2), 0:32]
                s = jnp.dot(up32(kc), q, preferred_element_type=F32)
                sA[pl.ds(r0, C), :] = s
                return jnp.maximum(m8, jnp.max(s.reshape(C // 8, 8, TQ), axis=0))
            m8 = lax.fori_loop(0, NCH, p1, jnp.full((8, TQ), -jnp.inf, F32))
            m = jnp.max(m8, axis=0, keepdims=True)

            def p2(c, acc):
                r0 = pl.multiple_of(c * C, C)
                p = jnp.exp2(sA[pl.ds(r0, C), :] - m)
                return acc + jnp.dot(vs[h, :, pl.ds(r0, C)], rev8(p), preferred_element_type=F32)
            acc = lax.fori_loop(0, NCH, p2, jnp.zeros((VR, TQ), F32))
            pl.when((u & 1) == 0)(lambda: fin(u, acc, False))
            pl.when((u & 1) == 1)(lambda: fin(u, acc, True))
            return carry
        lax.fori_loop(0, NU, unit, 0)

    def outp(t, carry):
        for hf in range(NH):
            cols = pl.ds(pl.multiple_of(t * TQ + hf * TH, TH), TH)
            o = ot[:, cols].T.astype(BF16)
            y = jnp.dot(o, wo_v[...], preferred_element_type=F32)
            out_v[cols, :] = y.astype(BF16)
            pltpu.make_async_copy(out_v.at[cols, :], out_hbm.at[cols, :], osems.at[NH * t + hf]).start()
        return carry
    lax.fori_loop(0, NQ, outp, 0)
    for i in range(NQ * NH):
        rows = pl.ds(i * TH, TH)
        pltpu.make_async_copy(out_v.at[rows, :], out_hbm.at[rows, :], osems.at[i]).wait()


@jax.jit
def pallas_gated_mix__mha_block__linear_kernel_hedgehog__prompt_kernel(
        A_x, A_wqkv, A_wo, B_x, B_wqkv, B_w_phi, B_wo, gate_w):
    x = A_x.reshape(S, D)
    wphi = jnp.transpose(B_w_phi, (1, 2, 0))
    any_spec = pl.BlockSpec(memory_space=pl.ANY)
    out = pl.pallas_call(
        _kernel,
        out_shape=jax.ShapeDtypeStruct((S, D), BF16),
        in_specs=[any_spec] * 7,
        out_specs=any_spec,
        scratch_shapes=[
            pltpu.VMEM((DH, DH, H), BF16), pltpu.VMEM((D,), BF16),
            pltpu.VMEM((S, D), BF16), pltpu.VMEM((D, D), BF16), pltpu.VMEM((D, D), BF16), pltpu.VMEM((D, D), BF16),
            pltpu.VMEM((D, 3 * D), BF16), pltpu.VMEM((2 * D, D), BF16),
            pltpu.VMEM((D // 2, D), U32), pltpu.VMEM((LTR // 2, D), U32),
            pltpu.VMEM((24, D), F32), pltpu.VMEM((8, 80, 256), BF16),
            pltpu.VMEM((H, 16, S), U32), pltpu.VMEM((8, S // 2, 128), U32), pltpu.VMEM((H, S // 2, 128), U32), pltpu.VMEM((H, VR, S), F32),
            pltpu.VMEM((D, S), F32), pltpu.VMEM((D, S), F32), pltpu.VMEM((D, S), F32), pltpu.VMEM((D, S), F32),
            pltpu.VMEM((D, S), F32), pltpu.VMEM((8, S), F32),
            pltpu.VMEM((16, 8, TP), F32), pltpu.VMEM((16, 8, TP), F32),
            pltpu.VMEM((S, TQ), F32), pltpu.VMEM((8, TQ), F32), pltpu.VMEM((VR, TQ), F32),
            pltpu.VMEM((C, TQ), F32),
            pltpu.VMEM((2 * D, S), F32), pltpu.VMEM((S, D), BF16), pltpu.VMEM((D, TP), F32),
            pltpu.SemaphoreType.DMA((18,)), pltpu.SemaphoreType.DMA((NQ * NH,)),
        ],
        compiler_params=pltpu.CompilerParams(vmem_limit_bytes=110 * 1024 * 1024),
    )(x, A_wqkv, A_wo, B_wqkv, wphi, B_wo, gate_w)
    return out.reshape(1, S, D)
```
